```python
import jax
import jax.numpy as jnp

def _softmax(x, axis=-1):
    return jax.nn.softmax(x, axis=axis)
def _gelu(x):
    return jax.nn.gelu(x, approximate=True)
def _silu(x):
    return jax.nn.silu(x)
def _sigmoid(x):
    return jax.nn.sigmoid(x)
def _layernorm(x, axis=-1, eps=1e-5):
    m = jnp.mean(x, axis=axis, keepdims=True)
    v = jnp.var(x, axis=axis, keepdims=True)
    return (x - m) / jnp.sqrt(v + eps)
def _scatter_add(tgt, idx, src, axis=0):
    return tgt.at[idx].add(src)
def _segment_sum(src, seg, n):
    return jax.ops.segment_sum(src, seg, n)
class _Rng:
    def __init__(self, key):
        self._k = key
    def _next(self):
        self._k, sub = jax.random.split(self._k)
        return sub
    def normal(self, shape):
        return jax.random.normal(self._next(), shape, dtype=jnp.bfloat16)
    def randint(self, lo, hi, shape):
        return jax.random.randint(self._next(), shape, lo, hi, dtype=jnp.int32)
    def uniform(self, shape, lo=0.0, hi=1.0):
        return jax.random.uniform(self._next(), shape, jnp.bfloat16, lo, hi)
    def permutation(self, n):
        return jax.random.permutation(self._next(), n)


kernel_name = 'standalone__modern_conv_block_convnext_v2__vision'

def setup_inputs():
    _rng = _Rng(jax.random.key(int.from_bytes(__import__("os").urandom(4), "little")))
    _w = (lambda a: (lambda t: t.astype(jnp.bfloat16) if jnp.issubdtype(t.dtype, jnp.floating) else t)(jnp.asarray(a)))
    H = W = 512
    C = 96
    K = 3
    return {
        "x": _w((lambda *s: _rng.normal(s) * 0.05)(1, H, W, C)),
        "dw": _w((lambda *s: _rng.normal(s) * 0.05)(K, K, C)),
        "w1": _w((lambda *s: _rng.normal(s) * 0.05)(C, 4 * C)),
        "w2": _w((lambda *s: _rng.normal(s) * 0.05)(4 * C, C)),
        "grn_gamma": _w((lambda *s: _rng.normal(s) * 0.05)(4 * C)),
        "grn_beta": _w((lambda *s: _rng.normal(s) * 0.05)(4 * C)),
    }

def reference(x, dw, w1, w2, grn_gamma, grn_beta):
    B, H, W, C = x.shape
    K = dw.shape[0]
    pad = K // 2
    xp = jnp.pad(x, ((0,0),(pad,pad),(pad,pad),(0,0)))
    out = jnp.zeros_like(x)
    for i in range(K):
        for j in range(K):
            out = out + xp[:, i:i+H, j:j+W, :] * dw[i, j][None, None, None, :]
    h = _layernorm(out, axis=-1)
    h = jnp.einsum('bhwc,ce->bhwe', h, w1)
    h = _gelu(h)
    gx = jnp.sqrt((h * h).sum(axis=(1, 2), keepdims=True) + 1e-6)
    nx = gx / (gx.mean(axis=-1, keepdims=True) + 1e-6)
    h = grn_gamma * (h * nx) + grn_beta + h
    h = jnp.einsum('bhwe,ec->bhwc', h, w2)
    return x + h
```

```python
import functools
import math

import jax
import jax.numpy as jnp
import jax.experimental.pallas as pl
import jax.experimental.pallas.tpu as pltpu

RB = 8
NREC = 3
VMEM_LIMIT = 127 * 1024 * 1024
CG = 96

_C0 = math.sqrt(2.0 / math.pi)
_K = (_C0 * 0.044715) ** (1.0 / 3.0)
_B = _C0 / _K
F32 = jnp.float32
BF16 = jnp.bfloat16


def _kernel(x_hbm, dw_ref, w1_ref, w2t_ref, gamma_ref, beta_ref, o_hbm,
            xbuf, obuf, hbuf, dwb, w1t, w2s, bias, ssq, isem, osem):
    H, C, W = x_hbm.shape
    E = w1_ref.shape[1]
    NB = H // RB
    NST = RB - NREC
    rec_rows = list(range(1, 1 + NREC))
    st_rows = [r for r in range(RB) if r not in rec_rows]

    def main_copy(t, s):
        return pltpu.make_async_copy(x_hbm.at[pl.ds(t * RB, RB)], xbuf.at[s, pl.ds(1, RB)], isem.at[s, 0])

    def top_copy(t, s):
        return pltpu.make_async_copy(x_hbm.at[pl.ds(jnp.maximum(t * RB - 1, 0), 1)], xbuf.at[s, pl.ds(0, 1)], isem.at[s, 1])

    def bot_copy(t, s):
        return pltpu.make_async_copy(x_hbm.at[pl.ds(jnp.minimum(t * RB + RB, H - 1), 1)], xbuf.at[s, pl.ds(RB + 1, 1)], isem.at[s, 2])

    def out_copy(t, s):
        return pltpu.make_async_copy(obuf.at[s], o_hbm.at[pl.ds(t * RB, RB)], osem.at[s])

    main_copy(0, 0).start()
    top_copy(0, 0).start()
    bot_copy(0, 0).start()

    eye = (jax.lax.broadcasted_iota(jnp.int32, (C, C), 0) == jax.lax.broadcasted_iota(jnp.int32, (C, C), 1))
    for i in range(3):
        dwi = dw_ref[i].astype(F32)
        for j in range(3):
            col = jnp.sum(jnp.where(eye, dwi[j:j + 1, :], 0.0), axis=1, keepdims=True)
            dwb[i * 3 + j] = jnp.broadcast_to(col, (C, 128))
    w1p = jnp.concatenate([w1_ref[...].astype(F32), jnp.zeros((128 - C, E), F32)], axis=0)
    w1t[...] = w1p.T[:, :C].astype(BF16)
    ssq[...] = jnp.zeros_like(ssq)

    def conv_ln(s, rows):
        outs = [[] for _ in rows]
        for c0 in range(0, C, CG):
            lane = jax.lax.broadcasted_iota(jnp.int32, (CG, W), 1)
            xs = [xbuf[s, r, c0:c0 + CG, :].astype(F32) for r in range(rows[0], rows[-1] + 3)]
            wt = [jnp.tile(dwb[k, c0:c0 + CG, :], (1, W // 128)) for k in range(9)]
            for n in range(len(rows)):
                p = [xs[n] * wt[j] + xs[n + 1] * wt[3 + j] + xs[n + 2] * wt[6 + j] for j in range(3)]
                left = jnp.where(lane == 0, 0.0, pltpu.roll(p[0], 1, 1))
                right = jnp.where(lane == W - 1, 0.0, pltpu.roll(p[2], W - 1, 1))
                outs[n].append(left + p[1] + right)
        res = []
        for n in range(len(rows)):
            o = jnp.concatenate(outs[n], axis=0) if len(outs[n]) > 1 else outs[n][0]
            m = jnp.sum(o, axis=0, keepdims=True) * (1.0 / C)
            d = o - m
            v = jnp.sum(d * d, axis=0, keepdims=True) * (1.0 / C)
            res.append((d * (jax.lax.rsqrt(v + 1e-5) * _K)).astype(BF16))
        return res

    def mlp1(hn):
        z = jnp.dot(w1t[...], hn, preferred_element_type=F32)
        return z * (jnp.tanh(z * (z * z + _B)) + 1.0)

    def pass1(t, carry):
        s = t % 2

        @pl.when(t + 1 < NB)
        def _():
            main_copy(t + 1, 1 - s).start()
            top_copy(t + 1, 1 - s).start()
            bot_copy(t + 1, 1 - s).start()

        @pl.when(t + 1 == NB)
        def _():
            main_copy(0, 1 - s).start()

        main_copy(t, s).wait()
        top_copy(t, s).wait()
        bot_copy(t, s).wait()

        @pl.when(t == 0)
        def _():
            xbuf[s, 0] = jnp.zeros((C, W), BF16)

        @pl.when(t == NB - 1)
        def _():
            xbuf[s, RB + 1] = jnp.zeros((C, W), BF16)

        for r0 in range(0, RB, 2):
            hns = conv_ln(s, [r0, r0 + 1])
            for k, hn in enumerate(hns):
                r = r0 + k
                g = mlp1(hn)
                g2 = g * g
                acc = ssq[...]
                for q in range(W // 128):
                    acc = acc + g2[:, q * 128:(q + 1) * 128]
                ssq[...] = acc
                if r in st_rows:
                    hbuf[t * NST + st_rows.index(r)] = pltpu.bitcast(g.astype(BF16), jnp.int32)
        return carry

    jax.lax.fori_loop(0, NB, pass1, 0)

    inv = 1.0 / (2.0 * _K)
    tot = jnp.sum(ssq[...].T, axis=0, keepdims=True) * (inv * inv)
    gx = jnp.sqrt(tot + 1e-6)
    nx = gx / (jnp.sum(gx, axis=1, keepdims=True) * (1.0 / E) + 1e-6)
    sc = (gamma_ref[...].astype(F32) * nx + 1.0) * inv
    w2f = w2t_ref[...].astype(F32)
    w2s[...] = (w2f * sc).astype(BF16)
    bias[...] = jnp.broadcast_to(jnp.sum(w2f * beta_ref[...].astype(F32), axis=1, keepdims=True), (C, 128))

    def mlp2(s, r, g):
        y = jnp.dot(w2s[...], g, preferred_element_type=F32)
        y = y + jnp.tile(bias[...], (1, W // 128))
        obuf[s, r] = (xbuf[s, r + 1].astype(F32) + y).astype(BF16)

    def pass2(t, carry):
        s = t % 2

        @pl.when(t + 1 < NB)
        def _():
            main_copy(t + 1, 1 - s).start()

        main_copy(t, s).wait()

        @pl.when(t >= 2)
        def _():
            out_copy(t - 2, s).wait()

        hns = conv_ln(s, rec_rows) if rec_rows else []
        for k, r in enumerate(st_rows):
            mlp2(s, r, pltpu.bitcast(hbuf[t * NST + k], BF16))
        for r, hn in zip(rec_rows, hns):
            mlp2(s, r, mlp1(hn).astype(BF16))
        out_copy(t, s).start()
        return carry

    jax.lax.fori_loop(0, NB, pass2, 0)
    out_copy(NB - 2, NB % 2).wait()
    out_copy(NB - 1, (NB - 1) % 2).wait()


@jax.jit
def pallas_standalone__modern_conv_block_convnext_v2__vision_kernel(x, dw, w1, w2, grn_gamma, grn_beta):
    B, H, W, C = x.shape
    E = w1.shape[1]
    xt = jnp.transpose(x, (0, 1, 3, 2)).reshape(H, C, W)
    vmem = pl.BlockSpec(memory_space=pltpu.VMEM)
    hbm = pl.BlockSpec(memory_space=pl.ANY)
    out = pl.pallas_call(
        _kernel,
        out_shape=jax.ShapeDtypeStruct((H, C, W), x.dtype),
        in_specs=[hbm, vmem, vmem, vmem, vmem, vmem],
        out_specs=hbm,
        scratch_shapes=[
            pltpu.VMEM((2, RB + 2, C, W), BF16),
            pltpu.VMEM((2, RB, C, W), BF16),
            pltpu.VMEM((H // RB * (RB - NREC), E // 2, W), jnp.int32),
            pltpu.VMEM((9, C, 128), F32),
            pltpu.VMEM((E, C), BF16),
            pltpu.VMEM((C, E), BF16),
            pltpu.VMEM((C, 128), F32),
            pltpu.VMEM((E, 128), F32),
            pltpu.SemaphoreType.DMA((2, 3)),
            pltpu.SemaphoreType.DMA((2,)),
        ],
        compiler_params=pltpu.CompilerParams(vmem_limit_bytes=VMEM_LIMIT),
        name="convnext_v2_block",
    )(xt, dw, w1, w2.T, grn_gamma.reshape(1, E), grn_beta.reshape(1, E))
    return jnp.transpose(out.reshape(B, H, C, W), (0, 1, 3, 2))
```

```python
import math

import jax
import jax.numpy as jnp
import jax.experimental.pallas as pl
import jax.experimental.pallas.tpu as pltpu

RB = 8
NREC = 3
U1 = 1
U2 = 1
NX = 4
NO = 2
VMEM_LIMIT = 128 * 1024 * 1024
ST_AT = 3
B2_AT = (4, 5, 6, 7, 8, 9, 10, 11)
NC = 2
LAG1 = 4
SHA = 0
CV0, CV1 = 1, 27
XS_AT = 1
SEQ = 'us' + 'usd' * 11 + 'sd' + 's' * 7
LAG2 = 5
UM = 96
DBC = False
SCOPES = True

_C0 = math.sqrt(2.0 / math.pi)
_K = (_C0 * 0.044715) ** (1.0 / 3.0)
_B = _C0 / _K
F32 = jnp.float32
BF16 = jnp.bfloat16
I32 = jnp.int32


def _gelu(z):
    return z * (jnp.tanh(z * (z * z + _B)) + 1.0)


def _tree_sum(parts):
    while len(parts) > 1:
        parts = [parts[i] + parts[i + 1] for i in range(0, len(parts), 2)]
    return parts[0]


def _shifted(mid, left, right):
    lane = jax.lax.broadcasted_iota(I32, (8, 128), 1)
    zero = jnp.zeros((8, 128), mid[0].dtype)
    le = [zero] + [pltpu.roll(v, 1, 1) for v in left]
    ri = [pltpu.roll(v, 127, 1) for v in right] + [zero]
    n = len(mid)
    return ([jnp.where(lane == 0, le[c], le[c + 1]) for c in range(n)], mid,
            [jnp.where(lane == 127, ri[c + 1], ri[c]) for c in range(n)])


def _kernel(x_hbm, dw_ref, w1_ref, w2t_ref, gamma_ref, beta_ref, o_hbm,
            hbuf, dwb, w1t, ssq, isem, osem):
    H, C, W = x_hbm.shape
    E = w1_ref.shape[1]
    NB = H // RB
    NST = RB - NREC
    NG = C // 8
    NT = W // 128
    rec_rows = list(range(1, 1 + NREC))
    st_rows = [r for r in range(RB) if r not in rec_rows]

    def tiles(v):
        return [v[:, 128 * c:128 * c + 128] for c in range(NT)]

    def x_copy(xbuf, row, n, s, dst=0):
        return pltpu.make_async_copy(x_hbm.at[pl.ds(row, n)], xbuf.at[s, pl.ds(dst, n)], isem.at[s])

    def phase1(xbuf, sbuf, cbuf, rbuf, stat, hnbuf):
        R1 = RB * U1
        NI = H // R1
        x_copy(xbuf, 0, RB - 1, 0, 1).start()
        x_copy(xbuf, RB - 1, R1, 1).start()

        hw = hnbuf.bitcast(I32)
        eye = (jax.lax.broadcasted_iota(I32, (C, C), 0) == jax.lax.broadcasted_iota(I32, (C, C), 1))
        for i in range(3):
            dwi = dw_ref[i].astype(F32)
            for j in range(3):
                col = jnp.sum(jnp.where(eye, dwi[j:j + 1, :], 0.0), axis=1, keepdims=True)
                dwb[i * 3 + j] = jnp.broadcast_to(col, (C, 128))
        ro = jax.lax.broadcasted_iota(I32, (8, 128), 0)
        co = jax.lax.broadcasted_iota(I32, (8, 128), 1)
        for g in range(NG):
            halves = []
            for o in range(2):
                m = jnp.zeros((8, 128), F32)
                for i in range(3):
                    for j in range(3):
                        m = jnp.where(co == ro + (j * 32 + (i + o) * 8), dwb[i * 3 + j, g * 8:(g + 1) * 8, :], m)
                halves.append(m)
            hnbuf[16 + g // 6, 16 * (g % 6):16 * (g % 6) + 16, :] = jnp.concatenate(halves, axis=0).astype(BF16)
        w1p = jnp.concatenate([w1_ref[...].astype(F32), jnp.zeros((128 - C, E), F32)], axis=0)
        w1t[...] = w1p.T.astype(BF16)
        ssq[...] = jnp.zeros_like(ssq)

        pace = []
        sh, sh0 = (hw, 18) if SHA else (sbuf, 0)

        def sh_at(p, g, j, c):
            return sh0 + ((p % 4) * NG + g) * 2 + c // 2, pl.ds(8 * (3 * (c % 2) + j), 8)

        def shift(s, k, g):
            mid = tiles(pltpu.bitcast(xbuf[s, 2 * k:2 * k + 2, 8 * g:8 * g + 8, :].reshape(16, W), I32))
            for j, vs in enumerate(_shifted(mid, mid, mid)):
                for c in range(NT):
                    sh[sh_at(k, g, j, c)] = vs[c]

        def conv(q, g, acc, zero=0):
            rhs = jnp.concatenate([jnp.concatenate([sh[sh_at(p, g, j, c)] for c in range(NT)], axis=1)
                                   for j in range(3) for p in (q, q + 1)], axis=0)
            lhs = pltpu.bitcast(hw[16 + g // 6 + zero, 8 * (g % 6):8 * (g % 6) + 8, :], BF16)[:, :96]
            y = jnp.dot(lhs, pltpu.bitcast(rhs, BF16), preferred_element_type=F32)
            cbuf[q % NC, g] = y
            pace.append(y[0:8, 0:128])
            acc = (y, y * y) if acc is None else (acc[0] + y, acc[1] + y * y)
            if g == NG - 1:
                for n in range(2):
                    for i in range(2 * NT):
                        rbuf[n, 8 * i:8 * i + 8, :] = tiles(acc[n][8 * (i // NT):8 * (i // NT) + 8])[i % NT]
            return acc

        def ln_stats(q):
            m, m2 = [_tree_sum([rbuf[n, pl.ds(k, 8, stride=8), :] for k in range(8)]) * (1.0 / C) for n in range(2)]
            stat[q % 2, 0] = m
            stat[q % 2, 1] = jax.lax.rsqrt(jnp.maximum(m2 - m * m, 0.0) + 1e-5) * _K

        def ln_apply(q, i, zero=0):
            if len(pace) >= LAG1:
                stat[2, 0] = pace[-LAG1]
            r, c = 8 * (i // NT), 128 * (i % NT)
            d = (cbuf[q % NC, :, r:r + 8, c:c + 128] - stat[q % 2 + zero, 0, i:i + 1, :]) * stat[q % 2, 1, i:i + 1, :]
            hnbuf[(q % 2) * 8 + i] = d.reshape(C, 128).astype(BF16)

        def up(t, q, g):
            o, e0 = g // (NG // 2), (g % (NG // 2)) * 64
            lhs = pltpu.bitcast(w1t.bitcast(I32)[e0 // 2:e0 // 2 + 32, :], BF16)[:, :C]
            hn = pltpu.bitcast(jnp.concatenate([hw[(q % 2) * 8 + o * NT + c] for c in range(NT)], axis=1), BF16)
            a = _gelu(jnp.dot(lhs, hn, preferred_element_type=F32))
            ssq[e0:e0 + 64, :] += _tree_sum(tiles(a * a))
            b, r = divmod(2 * q + o, RB)
            if r in st_rows:
                for c in range(NT):
                    hbuf[(t * U1 + b) * NST + st_rows.index(r), c, e0:e0 + 64, :] = tiles(a)[c].astype(BF16)

        xbuf[0, 0] = jnp.zeros((C, W), BF16)
        x_copy(xbuf, 0, RB - 1, 0, 1).wait()
        for k in range(4):
            for g in range(NG):
                shift(0, k, g)
        acc = None
        for g in range(NG):
            acc = conv(0, g, acc)
        ln_stats(0)
        for i in range(2 * NT):
            if B2_AT[i] < NG:
                ln_apply(0, i)
        acc = None
        for g in range(NG):
            acc = conv(1, g, acc)

        def body(t, carry):
            s = (t + 1) % 2
            last = R1 - RB + 1
            pl.when(t + 2 < NI)(lambda: x_copy(xbuf, (t + 1) * R1 + RB - 1, R1, 1 - s).start())
            pl.when(t + 2 == NI)(lambda: x_copy(xbuf, H - last, last, 1 - s).start())
            pl.when(t + 1 < NI)(lambda: x_copy(xbuf, 0, R1, s).wait())

            @pl.when(t + 1 == NI)
            def _():
                x_copy(xbuf, 0, last, s).wait()
                xbuf[s, last] = jnp.zeros((C, W), BF16)

            zero = t >> 16
            pace.clear()
            for k in range(R1 // 2):
                acc = None
                for g in range(NG):
                    acc = conv(k + 2, g, acc, zero)
                    if g == ST_AT:
                        ln_stats(k + 1)
                    for i in range(2 * NT):
                        if B2_AT[i] % NG == g:
                            ln_apply(k + 1 - B2_AT[i] // NG, i, zero)
                    shift(s, k, g)
                    up(t, k, g)
            return carry

        with jax.named_scope('sc_p1'):
            jax.lax.fori_loop(0, NI, body, 0)

    def phase2(xbuf, obuf, cbuf, rbuf, stat, bias):
        AH = NX - U2
        for n in range(AH):
            x_copy(xbuf, n * RB, RB, n).start()
        WO = NREC * C
        AO = WO + C // 2

        def out_copy(b, s):
            return pltpu.make_async_copy(obuf.at[s], o_hbm.at[pl.ds(b * RB, RB)], osem.at[s])

        inv = 1.0 / (2.0 * _K)
        gx = jnp.sqrt(jnp.sum(ssq[...].T, axis=0, keepdims=True) * (inv * inv) + 1e-6)
        nx = gx / (jnp.sum(gx, axis=1, keepdims=True) * (1.0 / E) + 1e-6)
        sc = (gamma_ref[...].astype(F32).reshape(1, E) * nx + 1.0) * inv
        w2f = w2t_ref[...].astype(F32)
        cbuf[WO:WO + C // 2, 0:E] = pltpu.bitcast((w2f * sc).astype(BF16), F32)
        beta = beta_ref[...].astype(F32).reshape(1, E)
        bias[...] = jnp.broadcast_to(jnp.sum(w2f * beta, axis=1, keepdims=True), (C, 128))

        def conv(s, n, g, zero=0):
            xs = [xbuf[s, n + i, 8 * g:8 * g + 8, :].astype(F32) for i in range(3)]
            wt = [jnp.tile(dwb[k + (zero if k < 3 else 0), 8 * g:8 * g + 8, :], (1, NT)) for k in range(9)]
            p = [tiles(xs[0] * wt[j] + xs[1] * wt[3 + j] + xs[2] * wt[6 + j]) for j in range(3)]
            le, mid, ri = _shifted(p[1], p[0], p[2])
            y = jnp.concatenate([le[c] + mid[c] + ri[c] for c in range(NT)], axis=1)
            cbuf[n * C + 8 * g:n * C + 8 * g + 8, :] = y
            a1, a2 = (y, y * y) if g == 0 else (cbuf[AO:AO + 8, :] + y, cbuf[AO + 8:AO + 16, :] + y * y)
            if g < NG - 1:
                cbuf[AO:AO + 8, :] = a1
                cbuf[AO + 8:AO + 16, :] = a2
            else:
                for i, v in enumerate(tiles(a1) + tiles(a2)):
                    rbuf[8 * i:8 * i + 8, :] = v
                m = _tree_sum([rbuf[pl.ds(k, 8, stride=8), :] for k in range(8)]) * (1.0 / C)
                stat[n, 0] = m
                stat[n, 1] = jax.lax.rsqrt(jnp.maximum(pltpu.roll(m, NT, 0) - m * m, 0.0) + 1e-5) * _K

        cv_items = [((n + NREC - 1) % NREC, g) for n in range(NREC) for g in range(NG)]
        cv_at = [CV0 + i * (CV1 - CV0) // (len(cv_items) - 1) for i in range(len(cv_items))]
        x_copy(xbuf, 0, RB, 0).wait()
        for n, g in cv_items[NG:]:
            conv(0, n, g)

        def block(b, pace, zero):
            s, s1, so = b % NX, (b + 1) % NX, b % NO
            acts, ys = {}, {}
            base = len(pace)

            def up(n, c):
                hn = ((cbuf[n * C:(n + 1) * C, 128 * c:128 * c + 128] - stat[n, 0, c:c + 1, :])
                      * stat[n, 1, c:c + 1, :]).astype(BF16)
                parts = []
                for k in range(E // UM):
                    w = pltpu.bitcast(w1t.bitcast(I32)[UM // 2 * k:UM // 2 * (k + 1), :], BF16)[:, :C]
                    parts.append(_gelu(jnp.dot(w, hn, preferred_element_type=F32)))
                acts[n, c] = jnp.concatenate(parts, axis=0).astype(BF16)

            def down(r, c, a):
                i = len(pace) - base
                if len(pace) >= LAG2 and i in cv_at:
                    dwb[9, 0:8, :] = pace[-LAG2]
                for m, (n, g) in enumerate(cv_items):
                    if cv_at[m] == i:
                        assert ((n, NT - 1) in acts) if m >= NG else ((n, 0) not in acts)
                        conv(s1 if m >= NG else s, n, g, zero)
                if i == XS_AT:
                    pl.when(b + AH < NB)(lambda: x_copy(xbuf, (b + AH) * RB, RB, (b + AH) % NX).start())
                w = pltpu.bitcast(jnp.concatenate(
                    [cbuf[pl.ds(pl.multiple_of(WO + zero * 8, 8), 8), 0:E], cbuf[WO + 8:WO + C // 2, 0:E]], axis=0), BF16)
                y = jnp.dot(w, a, preferred_element_type=F32)
                pace.append(y[0:8])
                ys[r, c] = y
                if c % 2 == 1:
                    cols = slice(128 * c - 128, 128 * c + 128)
                    res = jnp.tile(bias[...], (1, 2)) + xbuf[s, r, :, cols].astype(F32)
                    obuf[so, r, :, cols] = (jnp.concatenate([ys[r, c - 1], y], axis=1) + res).astype(BF16)

            cnt = {'u': 0, 'd': 0, 's': 0}
            for op in SEQ:
                n, c = divmod(cnt[op], NT)
                cnt[op] += 1
                if op == 'u':
                    up(n, c)
                elif op == 'd':
                    down(rec_rows[n], c, acts[n, c])
                else:
                    down(st_rows[n], c, pltpu.bitcast(hbuf.bitcast(I32)[b * NST + n, c], BF16))
            assert cnt == {'u': NT * NREC, 'd': NT * NREC, 's': NT * NST}, cnt
            out_copy(b, so).start()

        def body(t, carry):
            for j in range(U2):
                b = t * U2 + j
                pl.when(b + 1 < NB)(lambda: x_copy(xbuf, 0, RB, (b + 1) % NX).wait())
                pl.when(b >= NO)(lambda: out_copy(0, b % NO).wait())
            pace = []
            for j in range(U2):
                block(t * U2 + j, pace, t >> 16)
            return carry

        with jax.named_scope('sc_p2'):
            jax.lax.fori_loop(0, NB // U2, body, 0)
        for n in range(NO):
            out_copy(0, n).wait()

    pl.run_scoped(
        phase1,
        pltpu.VMEM((2, RB * U1, C, W), BF16),
        pltpu.VMEM((1 if SHA else 8 * NG, C // 2, 128), I32),
        pltpu.VMEM((NC, NG, 16, W), F32),
        pltpu.VMEM((2, 64, 128), F32),
        pltpu.VMEM((3, 2, 8, 128), F32),
        pltpu.VMEM((18 + (8 * NG if SHA else 0), C, 128), BF16),
    )
    pl.run_scoped(
        phase2,
        pltpu.VMEM((NX, RB, C, W), BF16),
        pltpu.VMEM((NO, RB, C, W), BF16),
        pltpu.VMEM((NREC * C + C // 2 + 16, W), F32),
        pltpu.VMEM((64, 128), F32),
        pltpu.VMEM((NREC, 2, 8, 128), F32),
        pltpu.VMEM((C, 128), F32),
    )


@jax.jit
def pallas_standalone__modern_conv_block_convnext_v2__vision_kernel(x, dw, w1, w2, grn_gamma, grn_beta):
    B, H, W, C = x.shape
    E = w1.shape[1]
    xt = jnp.transpose(x, (0, 1, 3, 2)).reshape(H, C, W)
    vmem = pl.BlockSpec(memory_space=pltpu.VMEM)
    hbm = pl.BlockSpec(memory_space=pl.ANY)
    out = pl.pallas_call(
        _kernel,
        out_shape=jax.ShapeDtypeStruct((H, C, W), x.dtype),
        in_specs=[hbm, vmem, vmem, vmem, vmem, vmem],
        out_specs=hbm,
        scratch_shapes=[
            pltpu.VMEM((H // RB * (RB - NREC), W // 128, E, 128), BF16),
            pltpu.VMEM((10, C, 128), F32),
            pltpu.VMEM((E, 128), BF16),
            pltpu.VMEM((E, 128), F32),
            pltpu.SemaphoreType.DMA((NX,)),
            pltpu.SemaphoreType.DMA((NO,)),
        ],
        compiler_params=pltpu.CompilerParams(vmem_limit_bytes=VMEM_LIMIT, disable_bounds_checks=DBC),
        name="convnext_v2_block",
    )(xt, dw, w1, w2.T, grn_gamma, grn_beta)
    return jnp.transpose(out.reshape(B, H, C, W), (0, 1, 3, 2))
```

```python
import math

import jax
import jax.numpy as jnp
import jax.experimental.pallas as pl
import jax.experimental.pallas.tpu as pltpu

RB = 8
NREC = 3
U1 = 2
U2 = 1
NX = 4
NO = 2
VMEM_LIMIT = 128 * 1024 * 1024
ST_AT = 3
B2_AT = (4, 5, 6, 7, 8, 9, 10, 11)
NC = 2
LAG1 = 4
SHA = 0
KP1 = 1
KP2 = 0
RS = 9
CEN = 1
CV0, CV1 = 1, 27
XS_AT = (0, 0)
SEQ = 'us' + 'usd' * 11 + 'sd' + 's' * 7
LAG2 = 5
UM = 96
DBC = True
SCOPES = True

_C0 = math.sqrt(2.0 / math.pi)
_K = (_C0 * 0.044715) ** (1.0 / 3.0)
_B = _C0 / _K
F32 = jnp.float32
BF16 = jnp.bfloat16
I32 = jnp.int32


def _gelu(z):
    return z * (jnp.tanh(z * (z * z + _B)) + 1.0)


def _dot96(lhs, rhs, pad):
    if pad:
        rhs = jnp.concatenate([rhs, jnp.zeros((32, rhs.shape[1]), rhs.dtype)], axis=0)
    else:
        lhs = lhs[:, :96]
    return jnp.dot(lhs, rhs, preferred_element_type=F32)


def _tree_sum(parts):
    while len(parts) > 1:
        parts = [parts[i] + parts[i + 1] for i in range(0, len(parts), 2)]
    return parts[0]


def _shifted(mid, left, right):
    lane = jax.lax.broadcasted_iota(I32, (8, 128), 1)
    zero = jnp.zeros((8, 128), mid[0].dtype)
    le = [zero] + [pltpu.roll(v, 1, 1) for v in left]
    ri = [pltpu.roll(v, 127, 1) for v in right] + [zero]
    n = len(mid)
    return ([jnp.where(lane == 0, le[c], le[c + 1]) for c in range(n)], mid,
            [jnp.where(lane == 127, ri[c + 1], ri[c]) for c in range(n)])


def _kernel(x_hbm, dw_hbm, w1_hbm, w2t_hbm, gamma_hbm, beta_hbm, o_hbm,
            xbuf, hbuf, w1t, wbuf, tot, dw_ref, gamma_ref, beta_ref, isem, osem, wsem):
    H, C, W = x_hbm.shape
    E = w1_hbm.shape[1]
    NB = H // RB
    NST = RB - NREC
    NG = C // 8
    NT = W // 128
    rec_rows = list(range(1, 1 + NREC))
    st_rows = [r for r in range(RB) if r not in rec_rows]

    def tiles(v):
        return [v[:, 128 * c:128 * c + 128] for c in range(NT)]

    def x_copy(row, n, s, dst=0):
        return pltpu.make_async_copy(x_hbm.at[pl.ds(row, n)], xbuf.at[pl.ds(s * RB + dst, n)], isem.at[s])

    def x_slot(b):
        return (b + U1) % NX

    dw_copy = pltpu.make_async_copy(dw_hbm, dw_ref, wsem.at[0])
    w1_copy = pltpu.make_async_copy(w1_hbm, wbuf, wsem.at[1])
    late_copies = [pltpu.make_async_copy(w2t_hbm, wbuf, wsem.at[0]),
                   pltpu.make_async_copy(gamma_hbm, gamma_ref, wsem.at[1]),
                   pltpu.make_async_copy(beta_hbm, beta_ref, wsem.at[2])]

    def tap_columns():
        eye = (jax.lax.broadcasted_iota(I32, (C, C), 0) == jax.lax.broadcasted_iota(I32, (C, C), 1))
        rows = [dw_ref[i].astype(F32) for i in range(3)]
        return [jnp.sum(jnp.where(eye, rows[i][j:j + 1, :], 0.0), axis=1, keepdims=True)
                for i in range(3) for j in range(3)]

    def phase1(sbuf, cbuf, rbuf, stat, hnbuf, ssq):
        R1 = RB * U1
        NI = H // R1
        dw_copy.start()
        w1_copy.start()
        x_copy(0, RB - 1, 0, 1).start()
        x_copy(RB - 1, R1, U1).start()

        hw = hnbuf.bitcast(I32)
        dw_copy.wait()
        taps = tap_columns()
        ro = jax.lax.broadcasted_iota(I32, (8, 128), 0)
        co = jax.lax.broadcasted_iota(I32, (8, 128), 1)
        for g in range(NG):
            halves = []
            for o in range(2):
                m = jnp.zeros((8, 128), F32)
                for i in range(3):
                    for j in range(3):
                        m = jnp.where(co == ro + (j * 32 + (i + o) * 8), taps[i * 3 + j][g * 8:(g + 1) * 8], m)
                halves.append(m)
            hnbuf[16 + g // 6, 16 * (g % 6):16 * (g % 6) + 16, :] = jnp.concatenate(halves, axis=0).astype(BF16)
        ssq[...] = jnp.zeros_like(ssq)

        pace = []
        sh, sh0 = (hw, 18) if SHA else (sbuf, 0)

        def sh_at(p, g, j, c):
            return sh0 + ((p % 4) * NG + g) * 2 + c // 2, pl.ds(8 * (3 * (c % 2) + j), 8)

        def shift(s, k, g):
            mid = tiles(pltpu.bitcast(xbuf[pl.ds(s * RB + 2 * k, 2), 8 * g:8 * g + 8, :].reshape(16, W), I32))
            for j, vs in enumerate(_shifted(mid, mid, mid)):
                for c in range(NT):
                    sh[sh_at(k, g, j, c)] = vs[c]

        def conv(q, g, acc, zero=0):
            rhs = jnp.concatenate([jnp.concatenate([sh[sh_at(p, g, j, c)] for c in range(NT)], axis=1)
                                   for j in range(3) for p in (q, q + 1)], axis=0)
            lhs = pltpu.bitcast(hw[16 + g // 6 + zero, 8 * (g % 6):8 * (g % 6) + 8, :], BF16)
            y = _dot96(lhs, pltpu.bitcast(rhs, BF16), KP1)
            cbuf[q % NC, g] = y
            pace.append(y[0:8, 0:128])
            acc = (y, y * y) if acc is None else (acc[0] + y, acc[1] + y * y)
            if g == NG - 1:
                for n in range(2):
                    for i in range(2 * NT):
                        rbuf[n, RS * i:RS * i + 8, :] = tiles(acc[n][8 * (i // NT):8 * (i // NT) + 8])[i % NT]
            return acc

        def ln_stats(q):
            m, m2 = [_tree_sum([rbuf[n, pl.ds(k, 8, stride=RS), :] for k in range(8)]) * (1.0 / C) for n in range(2)]
            stat[q % 2, 0] = m
            stat[q % 2, 1] = jax.lax.rsqrt(jnp.maximum(m2 - m * m, 0.0) + 1e-5) * _K

        def ln_apply(q, i, zero=0):
            if len(pace) >= LAG1:
                stat[2, 0] = pace[-LAG1]
            r, c = 8 * (i // NT), 128 * (i % NT)
            d = cbuf[q % NC, :, r:r + 8, c:c + 128]
            if not CEN:
                d = d - stat[q % 2 + zero, 0, i:i + 1, :]
            d = d * stat[q % 2 + (zero if CEN else 0), 1, i:i + 1, :]
            hnbuf[(q % 2) * 8 + i] = d.reshape(C, 128).astype(BF16)

        def up(t, q, g):
            o, e0 = g // (NG // 2), (g % (NG // 2)) * 64
            lhs = pltpu.bitcast(w1t.bitcast(I32)[e0 // 2:e0 // 2 + 32, :], BF16)
            hn = pltpu.bitcast(jnp.concatenate([hw[(q % 2) * 8 + o * NT + c] for c in range(NT)], axis=1), BF16)
            a = _gelu(_dot96(lhs, hn, KP1))
            ssq[e0:e0 + 64, :] += _tree_sum(tiles(a * a))
            b, r = divmod(2 * q + o, RB)
            if r in st_rows:
                for c in range(NT):
                    hbuf[(t * U1 + b) * NST + st_rows.index(r), c, e0:e0 + 64, :] = tiles(a)[c].astype(BF16)

        xbuf[0] = jnp.zeros((C, W), BF16)
        x_copy(0, RB - 1, 0, 1).wait()
        w1_copy.wait()
        w1f = wbuf[...].astype(F32)
        if CEN:
            w1f = w1f - jnp.sum(w1f, axis=0, keepdims=True) * (1.0 / C)
        w1p = jnp.concatenate([w1f, jnp.zeros((128 - C, E), F32)], axis=0)
        w1t[...] = w1p.T.astype(BF16)
        for cp in late_copies:
            cp.start()
        for k in range(4):
            for g in range(NG):
                shift(0, k, g)
        acc = None
        for g in range(NG):
            acc = conv(0, g, acc)
        ln_stats(0)
        for i in range(2 * NT):
            if B2_AT[i] < NG:
                ln_apply(0, i)
        acc = None
        for g in range(NG):
            acc = conv(1, g, acc)

        def body(t, carry):
            s = ((t + 1) % 2) * U1
            last = R1 - RB + 1
            pl.when(t + 2 < NI)(lambda: x_copy((t + 1) * R1 + RB - 1, R1, U1 - s).start())
            pl.when(t + 2 == NI)(lambda: x_copy(H - last, last, U1 - s).start())
            pl.when(t + 1 < NI)(lambda: x_copy(0, R1, s).wait())

            @pl.when(t + 1 == NI)
            def _():
                x_copy(0, last, s).wait()
                xbuf[s * RB + last] = jnp.zeros((C, W), BF16)
                for n in range(U1):
                    x_copy(n * RB, RB, x_slot(n)).start()

            zero = t >> 16
            pace.clear()
            for k in range(R1 // 2):
                acc = None
                for g in range(NG):
                    acc = conv(k + 2, g, acc, zero)
                    if g == ST_AT:
                        ln_stats(k + 1)
                    for i in range(2 * NT):
                        if B2_AT[i] % NG == g:
                            ln_apply(k + 1 - B2_AT[i] // NG, i, zero)
                    shift(s, k, g)
                    up(t, k, g)
            return carry

        with jax.named_scope('sc_p1'):
            jax.lax.fori_loop(0, NI, body, 0)
        for cp in late_copies:
            cp.wait()
        x_copy(0, RB, x_slot(0)).wait()
        tot[...] = jnp.sum(ssq[...].T, axis=0, keepdims=True)

    def phase2(obuf, cbuf, rbuf, stat, bias, dwb):
        AH = NX - U2
        for n in range(U1, AH):
            x_copy(n * RB, RB, x_slot(n)).start()
        WO = NREC * C
        AO = WO + C // 2

        def out_copy(b, s):
            return pltpu.make_async_copy(obuf.at[s], o_hbm.at[pl.ds(b * RB, RB)], osem.at[s])

        inv = 1.0 / (2.0 * _K)
        gx = jnp.sqrt(tot[...] * (inv * inv) + 1e-6)
        nx = gx / (jnp.sum(gx, axis=1, keepdims=True) * (1.0 / E) + 1e-6)
        sc = (gamma_ref[...].astype(F32).reshape(1, E) * nx + 1.0) * inv
        for k, col in enumerate(tap_columns()):
            dwb[k * NG:(k + 1) * NG] = jnp.broadcast_to(col, (C, 128)).reshape(NG, 8, 128)
        w2f = wbuf[...].astype(F32)
        cbuf[WO:WO + C // 2, 0:E] = pltpu.bitcast((w2f * sc).astype(BF16), F32)
        beta = beta_ref[...].astype(F32).reshape(1, E)
        bias[...] = jnp.broadcast_to(jnp.sum(w2f * beta, axis=1, keepdims=True), (C, 128))

        def conv(s, n, g, zero=0):
            xs = [xbuf[s * RB + n + i, 8 * g:8 * g + 8, :].astype(F32) for i in range(3)]
            wt = [jnp.tile(dwb[k * NG + g + (zero if k < 3 else 0)], (1, NT)) for k in range(9)]
            p = [tiles(xs[0] * wt[j] + xs[1] * wt[3 + j] + xs[2] * wt[6 + j]) for j in range(3)]
            le, mid, ri = _shifted(p[1], p[0], p[2])
            y = jnp.concatenate([le[c] + mid[c] + ri[c] for c in range(NT)], axis=1)
            cbuf[n * C + 8 * g:n * C + 8 * g + 8, :] = y
            a1, a2 = (y, y * y) if g == 0 else (cbuf[AO:AO + 8, :] + y, cbuf[AO + 8:AO + 16, :] + y * y)
            if g < NG - 1:
                cbuf[AO:AO + 8, :] = a1
                cbuf[AO + 8:AO + 16, :] = a2
            else:
                for i, v in enumerate(tiles(a1) + tiles(a2)):
                    rbuf[RS * i:RS * i + 8, :] = v
                m = _tree_sum([rbuf[pl.ds(k, 8, stride=RS), :] for k in range(8)]) * (1.0 / C)
                stat[n, 0] = m
                stat[n, 1] = jax.lax.rsqrt(jnp.maximum(pltpu.roll(m, NT, 0) - m * m, 0.0) + 1e-5) * _K

        cv_items = [((n + NREC - 1) % NREC, g) for n in range(NREC) for g in range(NG)]
        cv_at = [CV0 + i * (CV1 - CV0) // (len(cv_items) - 1) for i in range(len(cv_items))]
        for n, g in cv_items[NG:]:
            conv(x_slot(0), n, g)

        def block(b0, b, pace, zero):
            s, s1, so = x_slot(b), x_slot(b + 1), b % NO
            acts, ys = {}, {}
            base = len(pace)

            def up(n, c):
                hn = ((cbuf[n * C:(n + 1) * C, 128 * c:128 * c + 128] if CEN else cbuf[n * C:(n + 1) * C, 128 * c:128 * c + 128] - stat[n, 0, c:c + 1, :])
                      * stat[n, 1, c:c + 1, :]).astype(BF16)
                parts = []
                for k in range(E // UM):
                    w = pltpu.bitcast(w1t.bitcast(I32)[UM // 2 * k:UM // 2 * (k + 1), :], BF16)
                    parts.append(_gelu(_dot96(w, hn, KP2)))
                acts[n, c] = jnp.concatenate(parts, axis=0).astype(BF16)

            def down(r, c, a):
                i = len(pace) - base
                if len(pace) >= LAG2 and i in cv_at:
                    dwb[9 * NG] = pace[-LAG2]
                for m, (n, g) in enumerate(cv_items):
                    if cv_at[m] == i:
                        assert ((n, NT - 1) in acts) if m >= NG else ((n, 0) not in acts)
                        conv(s1 if m >= NG else s, n, g, zero)
                for j in range(U2):
                    if len(pace) == XS_AT[j]:
                        nb = b0 + AH + j
                        pl.when(nb < NB)(lambda: x_copy(nb * RB, RB, x_slot(nb)).start())
                w = pltpu.bitcast(jnp.concatenate(
                    [cbuf[pl.ds(pl.multiple_of(WO + zero * 8, 8), 8), 0:E], cbuf[WO + 8:WO + C // 2, 0:E]], axis=0), BF16)
                y = jnp.dot(w, a, preferred_element_type=F32)
                pace.append(y[0:8])
                ys[r, c] = y
                if c % 2 == 1:
                    cols = slice(128 * c - 128, 128 * c + 128)
                    res = jnp.tile(bias[...], (1, 2)) + xbuf[s * RB + r, :, cols].astype(F32)
                    obuf[so, r, :, cols] = (jnp.concatenate([ys[r, c - 1], y], axis=1) + res).astype(BF16)

            cnt = {'u': 0, 'd': 0, 's': 0}
            for op in SEQ:
                n, c = divmod(cnt[op], NT)
                cnt[op] += 1
                if op == 'u':
                    up(n, c)
                elif op == 'd':
                    down(rec_rows[n], c, acts[n, c])
                else:
                    down(st_rows[n], c, pltpu.bitcast(hbuf.bitcast(I32)[b * NST + n, c], BF16))
            assert cnt == {'u': NT * NREC, 'd': NT * NREC, 's': NT * NST}, cnt
            out_copy(b, so).start()

        def body(t, carry):
            for j in range(U2):
                b = t * U2 + j
                pl.when(b + 1 < NB)(lambda: x_copy(0, RB, x_slot(b + 1)).wait())
                pl.when(b >= NO)(lambda: out_copy(0, b % NO).wait())
            pace = []
            for j in range(U2):
                block(t * U2, t * U2 + j, pace, t >> 16)
            return carry

        with jax.named_scope('sc_p2'):
            jax.lax.fori_loop(0, NB // U2, body, 0)
        for n in range(NO):
            out_copy(0, n).wait()

    pl.run_scoped(
        phase1,
        pltpu.VMEM((1 if SHA else 8 * NG, C // 2, 128), I32),
        pltpu.VMEM((NC, NG, 16, W), F32),
        pltpu.VMEM((2, 8 * RS, 128), F32),
        pltpu.VMEM((3, 2, 8, 128), F32),
        pltpu.VMEM((18 + (8 * NG if SHA else 0), C, 128), BF16),
        pltpu.VMEM((E, 128), F32),
    )
    pl.run_scoped(
        phase2,
        pltpu.VMEM((NO, RB, C, W), BF16),
        pltpu.VMEM((NREC * C + C // 2 + 16, W), F32),
        pltpu.VMEM((8 * RS, 128), F32),
        pltpu.VMEM((NREC, 2, 8, 128), F32),
        pltpu.VMEM((C, 128), F32),
        pltpu.VMEM((9 * NG + 1, 8, 128), F32),
    )


@jax.jit
def pallas_standalone__modern_conv_block_convnext_v2__vision_kernel(x, dw, w1, w2, grn_gamma, grn_beta):
    B, H, W, C = x.shape
    E = w1.shape[1]
    xt = jnp.transpose(x, (0, 1, 3, 2)).reshape(H, C, W)
    vmem = pl.BlockSpec(memory_space=pltpu.VMEM)
    hbm = pl.BlockSpec(memory_space=pl.ANY)
    out = pl.pallas_call(
        _kernel,
        out_shape=jax.ShapeDtypeStruct((H, C, W), x.dtype),
        in_specs=[hbm] * 6,
        out_specs=hbm,
        scratch_shapes=[
            pltpu.VMEM((max(2 * U1, NX) * RB, C, W), BF16),
            pltpu.VMEM((H // RB * (RB - NREC), W // 128, E, 128), BF16),
            pltpu.VMEM((E, 128), BF16),
            pltpu.VMEM((C, E), BF16),
            pltpu.VMEM((1, E), F32),
            pltpu.VMEM(dw.shape, BF16),
            pltpu.VMEM((E,), BF16),
            pltpu.VMEM((E,), BF16),
            pltpu.SemaphoreType.DMA((NX,)),
            pltpu.SemaphoreType.DMA((NO,)),
            pltpu.SemaphoreType.DMA((3,)),
        ],
        compiler_params=pltpu.CompilerParams(vmem_limit_bytes=VMEM_LIMIT, disable_bounds_checks=DBC),
        name="convnext_v2_block",
    )(xt, dw, w1, w2.T, grn_gamma, grn_beta)
    return jnp.transpose(out.reshape(B, H, C, W), (0, 1, 3, 2))
```

```python
import math

import jax
import jax.numpy as jnp
import jax.experimental.pallas as pl
import jax.experimental.pallas.tpu as pltpu

RB = 8
NREC = 3
U1 = 2
U2 = 1
NX = 4
NO = 2
VMEM_LIMIT = 128 * 1024 * 1024
ST_AT = 3
B2_AT = (4, 5, 6, 7, 8, 9, 10, 11)
NC = 2
LAG1 = 5
SHA = 0
KP1 = 1
KP2 = 0
RS = 9
CEN = 1
CV0, CV1 = 1, 28
XS_AT = (14,)
NSB = 2
UPM = 64
SHD = 0
SEQ = 'us' + 'usd' * 11 + 'sd' + 's' * 7
LAG2 = 5
UM = 96
DBC = True
SCOPES = True

_C0 = math.sqrt(2.0 / math.pi)
_K = (_C0 * 0.044715) ** (1.0 / 3.0)
_B = _C0 / _K
F32 = jnp.float32
BF16 = jnp.bfloat16
I32 = jnp.int32


def _gelu(z):
    return z * (jnp.tanh(z * (z * z + _B)) + 1.0)


def _dot96(lhs, rhs, pad):
    if pad:
        rhs = jnp.concatenate([rhs, jnp.zeros((32, rhs.shape[1]), rhs.dtype)], axis=0)
    else:
        lhs = lhs[:, :96]
    return jnp.dot(lhs, rhs, preferred_element_type=F32)


def _walsh(a, c):
    p = a & c & 7
    return (1 - 2 * ((p ^ (p >> 1) ^ (p >> 2)) & 1)).astype(F32)


def _tree_sum(parts):
    while len(parts) > 1:
        parts = [parts[i] + parts[i + 1] if i + 1 < len(parts) else parts[i] for i in range(0, len(parts), 2)]
    return parts[0]


def _shifted(mid, left, right):
    lane = jax.lax.broadcasted_iota(I32, (8, 128), 1)
    zero = jnp.zeros((8, 128), mid[0].dtype)
    le = [zero] + [pltpu.roll(v, 1, 1) for v in left]
    ri = [pltpu.roll(v, 127, 1) for v in right] + [zero]
    n = len(mid)
    return ([jnp.where(lane == 0, le[c], le[c + 1]) for c in range(n)], mid,
            [jnp.where(lane == 127, ri[c + 1], ri[c]) for c in range(n)])


def _kernel(x_hbm, dw_hbm, w1_hbm, w2t_hbm, gamma_hbm, beta_hbm, o_hbm,
            xbuf, hbuf, w1t, wbuf, tot, dw_ref, gamma_ref, beta_ref, isem, osem, wsem):
    H, C, W = x_hbm.shape
    E = w1_hbm.shape[1]
    NB = H // RB
    NST = RB - NREC
    NG = C // 8
    NT = W // 128
    rec_rows = list(range(1, 1 + NREC))
    st_rows = [r for r in range(RB) if r not in rec_rows]

    def tiles(v):
        return [v[:, 128 * c:128 * c + 128] for c in range(NT)]

    def x_copy(row, n, s, dst=0):
        return pltpu.make_async_copy(x_hbm.at[pl.ds(row, n)], xbuf.at[pl.ds(s * RB + dst, n)], isem.at[s])

    def x_slot(b):
        return (b + U1) % NX

    dw_copy = pltpu.make_async_copy(dw_hbm, dw_ref, wsem.at[0])
    w1_copy = pltpu.make_async_copy(w1_hbm, wbuf, wsem.at[1])
    late_copies = [pltpu.make_async_copy(w2t_hbm, wbuf, wsem.at[0]),
                   pltpu.make_async_copy(gamma_hbm, gamma_ref, wsem.at[1]),
                   pltpu.make_async_copy(beta_hbm, beta_ref, wsem.at[2])]

    def tap_columns():
        eye = (jax.lax.broadcasted_iota(I32, (C, C), 0) == jax.lax.broadcasted_iota(I32, (C, C), 1))
        rows = [dw_ref[i].astype(F32) for i in range(3)]
        return [jnp.sum(jnp.where(eye, rows[i][j:j + 1, :], 0.0), axis=1, keepdims=True)
                for i in range(3) for j in range(3)]

    def phase1(sbuf, cbuf, rbuf, stat, hnbuf, ssq, w1h):
        R1 = RB * U1
        NI = H // R1
        dw_copy.start()
        w1_copy.start()
        x_copy(0, RB - 1, 0, 1).start()
        x_copy(RB - 1, R1, U1).start()

        hw = hnbuf.bitcast(I32)
        dw_copy.wait()
        taps = tap_columns()
        ro = jax.lax.broadcasted_iota(I32, (8, 128), 0)
        co = jax.lax.broadcasted_iota(I32, (8, 128), 1)
        for g in range(NG):
            halves = []
            for o in range(2):
                m = jnp.zeros((8, 128), F32)
                for i in range(3):
                    for j in range(3):
                        m = jnp.where(co == ro + (j * 32 + (i + o) * 8), taps[i * 3 + j][g * 8:(g + 1) * 8], m)
                halves.append(jnp.sum(m, axis=0, keepdims=True) * _walsh(ro, co))
            hnbuf[16 + g // 6, 16 * (g % 6):16 * (g % 6) + 16, :] = jnp.concatenate(halves, axis=0).astype(BF16)
        ssq[...] = jnp.zeros_like(ssq)

        pace = []
        sh, sh0 = (hw, 18) if SHA else (sbuf, 0)

        def sh_at(p, g, j, c):
            return sh0 + ((p % NSB) * NG + g) * 2 + c // 2, pl.ds(8 * (3 * (c % 2) + j), 8)

        def shift(s, k, g):
            mid = tiles(pltpu.bitcast(xbuf[pl.ds(s * RB + 2 * k, 2), 8 * g:8 * g + 8, :].reshape(16, W), I32))
            for j, vs in enumerate(_shifted(mid, mid, mid)):
                for c in range(NT):
                    sh[sh_at(k, g, j, c)] = vs[c]

        def conv(q, g, acc, zero=0):
            rhs = jnp.concatenate([jnp.concatenate([sh[sh_at(p, g, j, c)] for c in range(NT)], axis=1)
                                   for j in range(3) for p in (q, q + 1)], axis=0)
            lhs = pltpu.bitcast(hw[16 + g // 6 + zero, 8 * (g % 6):8 * (g % 6) + 8, :], BF16)
            y = _dot96(lhs, pltpu.bitcast(rhs, BF16), KP1)
            for i, v in enumerate(tiles(y[0:8]) + tiles(y[8:16])):
                cbuf[q % NC, g, RS * i:RS * i + 8, :] = v
            pace.append(y[0:8, 0:128])
            acc = y * y if acc is None else acc + y * y
            if g == NG - 1:
                for i, v in enumerate(tiles(acc[0:8]) + tiles(acc[8:16])):
                    rbuf[RS * i:RS * i + 8, :] = v
            return acc

        def ln_stats(q):
            m = _tree_sum([cbuf[q % NC, g, pl.ds(0, 8, stride=RS), :] for g in range(NG)]) * (1.0 / C)
            m2 = _tree_sum([rbuf[pl.ds(k, 8, stride=RS), :] for k in range(8)]) * (0.125 / C)
            stat[q % 2, 1] = jax.lax.rsqrt(jnp.maximum(m2 - m * m, 0.0) + 1e-5) * _K

        def ln_apply(q, i, zero=0):
            if len(pace) >= LAG1:
                stat[2, 0] = pace[-LAG1]
            r, c = 8 * (i // NT), 128 * (i % NT)
            d = cbuf[q % NC, :, RS * i:RS * i + 8, :]
            if not CEN:
                d = d - stat[q % 2 + zero, 0, i:i + 1, :]
            d = d * stat[q % 2 + (zero if CEN else 0), 1, i:i + 1, :]
            hnbuf[(q % 2) * 8 + i] = d.reshape(C, 128).astype(BF16)

        def up(t, q, g):
            o, e1 = g // (NG // 2), (g % (NG // 2) + 1) * 64
            if e1 % UPM:
                return
            e0 = e1 - UPM
            lhs = pltpu.bitcast(w1h.bitcast(I32)[e0 // 2:e1 // 2, :], BF16)
            hn = pltpu.bitcast(jnp.concatenate([hw[(q % 2) * 8 + o * NT + c] for c in range(NT)], axis=1), BF16)
            a = _gelu(_dot96(lhs, hn, KP1))
            ssq[e0:e1, :] += _tree_sum(tiles(a * a))
            b, r = divmod(2 * q + o, RB)
            if r in st_rows:
                for c in range(NT):
                    hbuf[(t * U1 + b) * NST + st_rows.index(r), c, e0:e1, :] = tiles(a)[c].astype(BF16)

        xbuf[0] = jnp.zeros((C, W), BF16)
        x_copy(0, RB - 1, 0, 1).wait()
        w1_copy.wait()
        w1f = wbuf[...].astype(F32)
        if CEN:
            w1f = w1f - jnp.sum(w1f, axis=0, keepdims=True) * (1.0 / C)
        w1p = jnp.concatenate([w1f, jnp.zeros((128 - C, E), F32)], axis=0)
        w1t[...] = w1p.T.astype(BF16)
        ra = jax.lax.broadcasted_iota(I32, (128, C), 0)
        ca = jax.lax.broadcasted_iota(I32, (128, C), 1)
        hd = jnp.where((ra >> 3) == (ca >> 3), _walsh(ra, ca) * 0.125, 0.0).astype(BF16)
        first = jax.lax.broadcasted_iota(I32, (128, E), 0)
        mu = jnp.sum(wbuf[...].astype(F32), axis=0, keepdims=True) * (1.0 / C)
        w1h[...] = (jnp.dot(hd, wbuf[...], preferred_element_type=F32)
                    - jnp.where(((first & 7) == 0) & (first < C), mu, 0.0)).T.astype(BF16)
        for cp in late_copies:
            cp.start()
        for k in range(2):
            for g in range(NG):
                shift(0, k, g)
        acc = None
        for g in range(NG):
            acc = conv(0, g, acc)
            shift(0, 2, g)
        ln_stats(0)
        for i in range(2 * NT):
            if B2_AT[i] < NG:
                ln_apply(0, i)
        acc = None
        for g in range(NG):
            acc = conv(1, g, acc)
            shift(0, 3, g)

        def body(t, carry):
            s = ((t + 1) % 2) * U1
            last = R1 - RB + 1
            pl.when(t + 2 < NI)(lambda: x_copy((t + 1) * R1 + RB - 1, R1, U1 - s).start())
            pl.when(t + 2 == NI)(lambda: x_copy(H - last, last, U1 - s).start())
            pl.when(t + 1 < NI)(lambda: x_copy(0, R1, s).wait())

            @pl.when(t + 1 == NI)
            def _():
                x_copy(0, last, s).wait()
                xbuf[s * RB + last] = jnp.zeros((C, W), BF16)
                for n in range(U1):
                    x_copy(n * RB, RB, x_slot(n)).start()

            zero = t >> 16
            pace.clear()
            for k in range(R1 // 2):
                acc = None
                for g in range(NG):
                    acc = conv(k + 2, g, acc, zero)
                    if g == ST_AT:
                        ln_stats(k + 1)
                    for i in range(2 * NT):
                        if B2_AT[i] % NG == g:
                            ln_apply(k + 1 - B2_AT[i] // NG, i, zero)
                    shift(s, k, g)
                    up(t, k, g)
            return carry

        with jax.named_scope('sc_p1'):
            jax.lax.fori_loop(0, NI, body, 0)
        for cp in late_copies:
            cp.wait()
        x_copy(0, RB, x_slot(0)).wait()
        tot[...] = jnp.sum(ssq[...].T, axis=0, keepdims=True)

    def phase2(obuf, cbuf, rbuf, stat, bias, dwb):
        AH = NX - U2
        for n in range(U1, AH):
            x_copy(n * RB, RB, x_slot(n)).start()
        WO = NREC * C
        AO = WO + C // 2

        def out_copy(b, s):
            return pltpu.make_async_copy(obuf.at[s], o_hbm.at[pl.ds(b * RB, RB)], osem.at[s])

        inv = 1.0 / (2.0 * _K)
        gx = jnp.sqrt(tot[...] * (inv * inv) + 1e-6)
        nx = gx / (jnp.sum(gx, axis=1, keepdims=True) * (1.0 / E) + 1e-6)
        sc = (gamma_ref[...].astype(F32).reshape(1, E) * nx + 1.0) * inv
        for k, col in enumerate(tap_columns()):
            dwb[k * NG:(k + 1) * NG] = jnp.broadcast_to(col, (C, 128)).reshape(NG, 8, 128)
        w2f = wbuf[...].astype(F32)
        cbuf[WO:WO + C // 2, 0:E] = pltpu.bitcast((w2f * sc).astype(BF16), F32)
        beta = beta_ref[...].astype(F32).reshape(1, E)
        bias[...] = jnp.broadcast_to(jnp.sum(w2f * beta, axis=1, keepdims=True), (C, 128))

        def conv(s, n, g, zero=0):
            xs = [xbuf[s * RB + n + i, 8 * g:8 * g + 8, :].astype(F32) for i in range(3)]
            wt = [jnp.tile(dwb[k * NG + g + (zero if k < 3 else 0)], (1, NT)) for k in range(9)]
            p = [tiles(xs[0] * wt[j] + xs[1] * wt[3 + j] + xs[2] * wt[6 + j]) for j in range(3)]
            le, mid, ri = _shifted(p[1], p[0], p[2])
            y = jnp.concatenate([le[c] + mid[c] + ri[c] for c in range(NT)], axis=1)
            cbuf[n * C + 8 * g:n * C + 8 * g + 8, :] = y
            a1, a2 = (y, y * y) if g == 0 else (cbuf[AO:AO + 8, :] + y, cbuf[AO + 8:AO + 16, :] + y * y)
            if g < NG - 1:
                cbuf[AO:AO + 8, :] = a1
                cbuf[AO + 8:AO + 16, :] = a2
            else:
                for i, v in enumerate(tiles(a1) + tiles(a2)):
                    rbuf[RS * i:RS * i + 8, :] = v
                m = _tree_sum([rbuf[pl.ds(k, 8, stride=RS), :] for k in range(8)]) * (1.0 / C)
                stat[n, 0] = m
                stat[n, 1] = jax.lax.rsqrt(jnp.maximum(pltpu.roll(m, NT, 0) - m * m, 0.0) + 1e-5) * _K

        cv_items = [((n + NREC - 1) % NREC, g) for n in range(NREC) for g in range(NG)]
        cv_at = [CV0 + i * (CV1 - CV0) // (len(cv_items) - 1) for i in range(len(cv_items))]
        for n, g in cv_items[NG:]:
            conv(x_slot(0), n, g)

        def block(b0, b, pace, zero):
            s, s1, so = x_slot(b), x_slot(b + 1), b % NO
            acts, ys = {}, {}
            base = len(pace)

            def up(n, c):
                hn = ((cbuf[n * C:(n + 1) * C, 128 * c:128 * c + 128] if CEN else cbuf[n * C:(n + 1) * C, 128 * c:128 * c + 128] - stat[n, 0, c:c + 1, :])
                      * stat[n, 1, c:c + 1, :]).astype(BF16)
                parts = []
                for k in range(E // UM):
                    w = pltpu.bitcast(w1t.bitcast(I32)[UM // 2 * k:UM // 2 * (k + 1), :], BF16)
                    parts.append(_gelu(_dot96(w, hn, KP2)))
                acts[n, c] = jnp.concatenate(parts, axis=0).astype(BF16)

            def down(r, c, a):
                i = len(pace) - base
                if len(pace) >= LAG2 and i in cv_at:
                    dwb[9 * NG] = pace[-LAG2]
                for m, (n, g) in enumerate(cv_items):
                    if cv_at[m] == i:
                        assert ((n, NT - 1) in acts) if m >= NG else ((n, 0) not in acts)
                        conv(s1 if m >= NG else s, n, g, zero)
                for j in range(U2):
                    if len(pace) == XS_AT[j]:
                        nb = b0 + AH + j
                        pl.when(nb < NB)(lambda: x_copy(nb * RB, RB, x_slot(nb)).start())
                w = pltpu.bitcast(jnp.concatenate(
                    [cbuf[pl.ds(pl.multiple_of(WO + zero * 8, 8), 8), 0:E], cbuf[WO + 8:WO + C // 2, 0:E]], axis=0), BF16)
                y = jnp.dot(w, a, preferred_element_type=F32)
                pace.append(y[0:8])
                ys[r, c] = y
                if c % 2 == 1:
                    cols = slice(128 * c - 128, 128 * c + 128)
                    res = jnp.tile(bias[...], (1, 2)) + xbuf[s * RB + r, :, cols].astype(F32)
                    obuf[so, r, :, cols] = (jnp.concatenate([ys[r, c - 1], y], axis=1) + res).astype(BF16)

            cnt = {'u': 0, 'd': 0, 's': 0}
            for op in SEQ:
                n, c = divmod(cnt[op], NT)
                cnt[op] += 1
                if op == 'u':
                    up(n, c)
                elif op == 'd':
                    down(rec_rows[n], c, acts[n, c])
                else:
                    down(st_rows[n], c, pltpu.bitcast(hbuf.bitcast(I32)[b * NST + n, c], BF16))
            assert cnt == {'u': NT * NREC, 'd': NT * NREC, 's': NT * NST}, cnt
            out_copy(b, so).start()

        def body(t, carry):
            for j in range(U2):
                b = t * U2 + j
                pl.when(b + 1 < NB)(lambda: x_copy(0, RB, x_slot(b + 1)).wait())
                pl.when(b >= NO)(lambda: out_copy(0, b % NO).wait())
            pace = []
            for j in range(U2):
                block(t * U2, t * U2 + j, pace, t >> 16)
            return carry

        with jax.named_scope('sc_p2'):
            jax.lax.fori_loop(0, NB // U2, body, 0)
        for n in range(NO):
            out_copy(0, n).wait()

    pl.run_scoped(
        phase1,
        pltpu.VMEM((1 if SHA else 2 * NSB * NG, C // 2, 128), I32),
        pltpu.VMEM((NC, NG, 8 * RS, 128), F32),
        pltpu.VMEM((8 * RS, 128), F32),
        pltpu.VMEM((3, 2, 8, 128), F32),
        pltpu.VMEM((18 + (8 * NG if SHA else 0), C, 128), BF16),
        pltpu.VMEM((E, 128), F32),
        pltpu.VMEM((E, 128), BF16),
    )
    pl.run_scoped(
        phase2,
        pltpu.VMEM((NO, RB, C, W), BF16),
        pltpu.VMEM((NREC * C + C // 2 + 16, W), F32),
        pltpu.VMEM((8 * RS, 128), F32),
        pltpu.VMEM((NREC, 2, 8, 128), F32),
        pltpu.VMEM((C, 128), F32),
        pltpu.VMEM((9 * NG + 1, 8, 128), F32),
    )


@jax.jit
def pallas_standalone__modern_conv_block_convnext_v2__vision_kernel(x, dw, w1, w2, grn_gamma, grn_beta):
    B, H, W, C = x.shape
    E = w1.shape[1]
    xt = jnp.transpose(x, (0, 1, 3, 2)).reshape(H, C, W)
    vmem = pl.BlockSpec(memory_space=pltpu.VMEM)
    hbm = pl.BlockSpec(memory_space=pl.ANY)
    out = pl.pallas_call(
        _kernel,
        out_shape=jax.ShapeDtypeStruct((H, C, W), x.dtype),
        in_specs=[hbm] * 6,
        out_specs=hbm,
        scratch_shapes=[
            pltpu.VMEM((max(2 * U1, NX) * RB, C, W), BF16),
            pltpu.VMEM((H // RB * (RB - NREC), W // 128, E, 128), BF16),
            pltpu.VMEM((E, 128), BF16),
            pltpu.VMEM((C, E), BF16),
            pltpu.VMEM((1, E), F32),
            pltpu.VMEM(dw.shape, BF16),
            pltpu.VMEM((E,), BF16),
            pltpu.VMEM((E,), BF16),
            pltpu.SemaphoreType.DMA((NX,)),
            pltpu.SemaphoreType.DMA((NO,)),
            pltpu.SemaphoreType.DMA((3,)),
        ],
        compiler_params=pltpu.CompilerParams(vmem_limit_bytes=VMEM_LIMIT, disable_bounds_checks=DBC),
        name="convnext_v2_block",
    )(xt, dw, w1, w2.T, grn_gamma, grn_beta)
    return jnp.transpose(out.reshape(B, H, C, W), (0, 1, 3, 2))
```

```python
import math

import jax
import jax.numpy as jnp
import jax.experimental.pallas as pl
import jax.experimental.pallas.tpu as pltpu

F32 = jnp.float32
BF16 = jnp.bfloat16
I32 = jnp.int32

RB = 8
NREC = 3
U1 = 2
NX = 4
NO = 2
RS = 9

LAG1 = 5
STATS_AT = 3
SCALE_AT = 4
SEQ = "us" + "usd" * 11 + "sd" + "s" * 7
LAG2 = 5
CONV_FROM, CONV_TO = 1, 28
FETCH_AT = 14

_C0 = math.sqrt(2.0 / math.pi)
_K = (_C0 * 0.044715) ** (1.0 / 3.0)
_B = _C0 / _K


def _gelu(z):
    return z * (jnp.tanh(z * (z * z + _B)) + 1.0)


def _ln_scale(mean, mean_sq):
    return jax.lax.rsqrt(jnp.maximum(mean_sq - mean * mean, 0.0) + 1e-5) * _K


def _dot(lhs, rhs):
    return jnp.dot(lhs, rhs, preferred_element_type=F32)


def _pad_rows(v):
    return jnp.concatenate([v, jnp.zeros((128 - v.shape[0], v.shape[1]), v.dtype)], axis=0)


def _walsh(a, c):
    p = a & c & 7
    return (1 - 2 * ((p ^ (p >> 1) ^ (p >> 2)) & 1)).astype(F32)


def _tree_sum(parts):
    while len(parts) > 1:
        parts = [parts[i] + parts[i + 1] if i + 1 < len(parts) else parts[i] for i in range(0, len(parts), 2)]
    return parts[0]


def _tiles(v):
    return [v[:, c:c + 128] for c in range(0, v.shape[1], 128)]


def _neighbours(left, right):
    lane = jax.lax.broadcasted_iota(I32, (8, 128), 1)
    zero = jnp.zeros((8, 128), left[0].dtype)
    le = [zero] + [pltpu.roll(v, 1, 1) for v in left]
    ri = [pltpu.roll(v, 127, 1) for v in right] + [zero]
    return ([jnp.where(lane == 0, le[c], le[c + 1]) for c in range(len(left))],
            [jnp.where(lane == 127, ri[c + 1], ri[c]) for c in range(len(right))])


def _kernel(x_hbm, dw_hbm, w1_hbm, w2t_hbm, gamma_hbm, beta_hbm, o_hbm,
            xbuf, hbuf, w1t, wbuf, total, dw_ref, gamma_ref, beta_ref, isem, osem, wsem):
    H, C, W = x_hbm.shape
    E = w1_hbm.shape[1]
    NB = H // RB
    NG = C // 8
    NT = W // 128
    NST = RB - NREC
    rec_rows = list(range(1, 1 + NREC))
    st_rows = [r for r in range(RB) if r not in rec_rows]

    def x_copy(row, n, slot, dst=0):
        return pltpu.make_async_copy(x_hbm.at[pl.ds(row, n)], xbuf.at[pl.ds(slot * RB + dst, n)], isem.at[slot])

    def x_slot(b):
        return (b + U1) % NX

    def block_copy(b):
        return x_copy(b * RB, RB, x_slot(b))

    def tap_columns():
        eye = jax.lax.broadcasted_iota(I32, (C, C), 0) == jax.lax.broadcasted_iota(I32, (C, C), 1)
        rows = [dw_ref[i].astype(F32) for i in range(3)]
        return [jnp.sum(jnp.where(eye, rows[i][j:j + 1, :], 0.0), axis=1, keepdims=True)
                for i in range(3) for j in range(3)]

    def pass1(sbuf, cbuf, rbuf, scale, hnbuf, ssq, w1h):
        R1 = RB * U1
        NI = H // R1
        LAST = R1 - RB + 1
        TAPS = 4 * NT
        hw = hnbuf.bitcast(I32)
        pace = []

        def chunk_copy(t, n=R1):
            return x_copy(t * R1 + RB - 1, n, ((t + 1) % 2) * U1)

        dw_copy = pltpu.make_async_copy(dw_hbm, dw_ref, wsem.at[0])
        w1_copy = pltpu.make_async_copy(w1_hbm, wbuf, wsem.at[1])
        head_copy = x_copy(0, RB - 1, 0, 1)
        late_copies = [pltpu.make_async_copy(w2t_hbm, wbuf, wsem.at[0]),
                       pltpu.make_async_copy(gamma_hbm, gamma_ref, wsem.at[1]),
                       pltpu.make_async_copy(beta_hbm, beta_ref, wsem.at[2])]
        for cp in (dw_copy, w1_copy, head_copy, chunk_copy(0)):
            cp.start()

        dw_copy.wait()
        taps = tap_columns()
        ro = jax.lax.broadcasted_iota(I32, (8, 128), 0)
        co = jax.lax.broadcasted_iota(I32, (8, 128), 1)
        for g in range(NG):
            halves = []
            for o in range(2):
                m = jnp.zeros((8, 128), F32)
                for i in range(3):
                    for j in range(3):
                        m = jnp.where(co == ro + (j * 32 + (i + o) * 8), taps[i * 3 + j][g * 8:(g + 1) * 8], m)
                halves.append(jnp.sum(m, axis=0, keepdims=True) * _walsh(ro, co))
            hnbuf[TAPS + g // 6, 16 * (g % 6):16 * (g % 6) + 16, :] = jnp.concatenate(halves, axis=0).astype(BF16)
        ssq[...] = jnp.zeros_like(ssq)
        xbuf[0] = jnp.zeros((C, W), BF16)

        head_copy.wait()
        w1_copy.wait()
        w1 = wbuf[...]
        mu = jnp.sum(w1.astype(F32), axis=0, keepdims=True) * (1.0 / C)
        w1t[...] = _pad_rows(w1.astype(F32) - mu).T.astype(BF16)
        ra = jax.lax.broadcasted_iota(I32, (128, C), 0)
        ca = jax.lax.broadcasted_iota(I32, (128, C), 1)
        unmix = jnp.where((ra >> 3) == (ca >> 3), _walsh(ra, ca) * 0.125, 0.0).astype(BF16)
        row = jax.lax.broadcasted_iota(I32, (128, E), 0)
        w1h[...] = (_dot(unmix, w1) - jnp.where(((row & 7) == 0) & (row < C), mu, 0.0)).T.astype(BF16)
        for cp in late_copies:
            cp.start()

        def s_at(p, g, j, c):
            return ((p % 2) * NG + g) * 2 + c // 2, pl.ds(8 * (3 * (c % 2) + j), 8)

        def shift(slot, k, g):
            two_rows = xbuf[pl.ds(slot * RB + 2 * k, 2), 8 * g:8 * g + 8, :].reshape(16, W)
            mid = _tiles(pltpu.bitcast(two_rows, I32))
            left, right = _neighbours(mid, mid)
            for j, vs in enumerate((left, mid, right)):
                for c in range(NT):
                    sbuf[s_at(k, g, j, c)] = vs[c]

        def conv(q, g, acc, zero=0):
            rhs = jnp.concatenate([jnp.concatenate([sbuf[s_at(p, g, j, c)] for c in range(NT)], axis=1)
                                   for j in range(3) for p in (q, q + 1)], axis=0)
            lhs = pltpu.bitcast(hw[TAPS + g // 6 + zero, 8 * (g % 6):8 * (g % 6) + 8, :], BF16)
            y = _dot(lhs, _pad_rows(pltpu.bitcast(rhs, BF16)))
            for i, v in enumerate(_tiles(y[0:8]) + _tiles(y[8:16])):
                cbuf[q % 2, g, RS * i:RS * i + 8, :] = v
            pace.append(y[0:8, 0:128])
            acc = y * y if acc is None else acc + y * y
            if g == NG - 1:
                for i, v in enumerate(_tiles(acc[0:8]) + _tiles(acc[8:16])):
                    rbuf[RS * i:RS * i + 8, :] = v
            return acc

        def ln_stats(q):
            mean = _tree_sum([cbuf[q % 2, g, pl.ds(0, 8, stride=RS), :] for g in range(NG)]) * (1.0 / C)
            mean_sq = _tree_sum([rbuf[pl.ds(k, 8, stride=RS), :] for k in range(8)]) * (0.125 / C)
            scale[q % 2] = _ln_scale(mean, mean_sq)

        def ln_apply(q, i, zero=0):
            if len(pace) >= LAG1:
                scale[2] = pace[-LAG1]
            d = cbuf[q % 2, :, RS * i:RS * i + 8, :] * scale[q % 2 + zero, i:i + 1, :]
            hnbuf[(q % 2) * 2 * NT + i] = d.reshape(C, 128).astype(BF16)

        def up(t, q, g):
            o, e0 = g // (NG // 2), (g % (NG // 2)) * 64
            lhs = pltpu.bitcast(w1h.bitcast(I32)[e0 // 2:e0 // 2 + 32, :], BF16)
            hn = jnp.concatenate([hw[((q % 2) * 2 + o) * NT + c] for c in range(NT)], axis=1)
            a = _gelu(_dot(lhs, _pad_rows(pltpu.bitcast(hn, BF16))))
            ssq[e0:e0 + 64, :] += _tree_sum(_tiles(a * a))
            b, r = divmod(2 * q + o, RB)
            if r in st_rows:
                for c, v in enumerate(_tiles(a)):
                    hbuf[(t * U1 + b) * NST + st_rows.index(r), c, e0:e0 + 64, :] = v.astype(BF16)

        for k in range(2):
            for g in range(NG):
                shift(0, k, g)
        for q in range(2):
            acc = None
            for g in range(NG):
                acc = conv(q, g, acc)
                shift(0, q + 2, g)
            if q == 0:
                ln_stats(0)
                for i in range(2 * NT):
                    ln_apply(0, i)

        def body(t, carry):
            slot = ((t + 1) % 2) * U1
            pl.when(t + 2 < NI)(lambda: chunk_copy(t + 1).start())
            pl.when(t + 2 == NI)(lambda: chunk_copy(NI - 1, LAST).start())
            pl.when(t + 1 < NI)(lambda: chunk_copy(t).wait())

            @pl.when(t + 1 == NI)
            def _():
                chunk_copy(NI - 1, LAST).wait()
                xbuf[slot * RB + LAST] = jnp.zeros((C, W), BF16)
                for b in range(U1):
                    block_copy(b).start()

            zero = t >> 16
            pace.clear()
            for k in range(R1 // 2):
                acc = None
                for g in range(NG):
                    acc = conv(k + 2, g, acc, zero)
                    if g == STATS_AT:
                        ln_stats(k + 1)
                    if g >= SCALE_AT:
                        ln_apply(k + 1, g - SCALE_AT, zero)
                    shift(slot, k, g)
                    up(t, k, g)
            return carry

        jax.lax.fori_loop(0, NI, body, 0)
        for cp in late_copies + [block_copy(0)]:
            cp.wait()
        total[...] = jnp.sum(ssq[...].T, axis=0, keepdims=True)

    def pass2(obuf, cbuf, rbuf, scale, bias, dwb):
        W2 = NREC * C
        ACC = W2 + C // 2
        for b in range(U1, NX - 1):
            block_copy(b).start()

        def out_copy(b):
            return pltpu.make_async_copy(obuf.at[b % NO], o_hbm.at[pl.ds(b * RB, RB)], osem.at[b % NO])

        inv = 1.0 / (2.0 * _K)
        gx = jnp.sqrt(total[...] * (inv * inv) + 1e-6)
        nx = gx / (jnp.sum(gx, axis=1, keepdims=True) * (1.0 / E) + 1e-6)
        grn = (gamma_ref[...].astype(F32).reshape(1, E) * nx + 1.0) * inv
        for k, col in enumerate(tap_columns()):
            dwb[k * NG:(k + 1) * NG] = jnp.broadcast_to(col, (C, 128)).reshape(NG, 8, 128)
        w2t = wbuf[...].astype(F32)
        cbuf[W2:ACC, 0:E] = pltpu.bitcast((w2t * grn).astype(BF16), I32)
        beta = beta_ref[...].astype(F32).reshape(1, E)
        bias[...] = jnp.broadcast_to(jnp.sum(w2t * beta, axis=1, keepdims=True), (C, 128))

        def conv(slot, n, g, zero=0):
            xs = [xbuf[slot * RB + n + i, 8 * g:8 * g + 8, :].astype(F32) for i in range(3)]
            wt = [jnp.tile(dwb[k * NG + g + (zero if k < 3 else 0)], (1, NT)) for k in range(9)]
            p = [_tiles(xs[0] * wt[j] + xs[1] * wt[3 + j] + xs[2] * wt[6 + j]) for j in range(3)]
            left, right = _neighbours(p[0], p[2])
            y = jnp.concatenate([left[c] + p[1][c] + right[c] for c in range(NT)], axis=1)
            cbuf[n * C + 8 * g:n * C + 8 * g + 8, :] = pltpu.bitcast(y, I32)
            sums = jnp.concatenate([y, y * y], axis=0)
            if g > 0:
                sums = pltpu.bitcast(cbuf[ACC:ACC + 16, :], F32) + sums
            if g < NG - 1:
                cbuf[ACC:ACC + 16, :] = pltpu.bitcast(sums, I32)
            else:
                for i, v in enumerate(_tiles(sums[0:8]) + _tiles(sums[8:16])):
                    rbuf[RS * i:RS * i + 8, :] = v
                m = _tree_sum([rbuf[pl.ds(k, 8, stride=RS), :] for k in range(8)]) * (1.0 / C)
                scale[n] = _ln_scale(m, pltpu.roll(m, NT, 0))

        convs = [((n + NREC - 1) % NREC, g) for n in range(NREC) for g in range(NG)]
        conv_at = [CONV_FROM + i * (CONV_TO - CONV_FROM) // (len(convs) - 1) for i in range(len(convs))]
        for n, g in convs[NG:]:
            conv(x_slot(0), n, g)

        def body(b, carry):
            pl.when(b + 1 < NB)(lambda: block_copy(b + 1).wait())
            pl.when(b >= NO)(lambda: out_copy(b - NO).wait())
            slot, slot1, zero = x_slot(b), x_slot(b + 1), b >> 16
            acts, ys, pace = {}, {}, []

            def up(n, c):
                y = pltpu.bitcast(cbuf[n * C:(n + 1) * C, 128 * c:128 * c + 128], F32)
                hn = (y * scale[n, c:c + 1, :]).astype(BF16)
                parts = []
                for k in range(E // C):
                    w = pltpu.bitcast(w1t.bitcast(I32)[C // 2 * k:C // 2 * (k + 1), :], BF16)[:, :C]
                    parts.append(_gelu(_dot(w, hn)))
                acts[n, c] = jnp.concatenate(parts, axis=0).astype(BF16)

            def down(r, c, a):
                i = len(pace)
                if i >= LAG2 and i in conv_at:
                    dwb[9 * NG] = pace[-LAG2]
                for m, (n, g) in enumerate(convs):
                    if conv_at[m] == i:
                        assert ((n, NT - 1) in acts) if m >= NG else ((n, 0) not in acts)
                        conv(slot1 if m >= NG else slot, n, g, zero)
                if i == FETCH_AT:
                    pl.when(b + NX - 1 < NB)(lambda: block_copy(b + NX - 1).start())
                w = jnp.concatenate([cbuf[pl.ds(pl.multiple_of(W2 + zero * 8, 8), 8), 0:E],
                                     cbuf[W2 + 8:ACC, 0:E]], axis=0)
                ys[r, c] = _dot(pltpu.bitcast(w, BF16), a)
                pace.append(ys[r, c][0:8])
                if c % 2 == 1:
                    cols = slice(128 * c - 128, 128 * c + 128)
                    res = jnp.tile(bias[...], (1, 2)) + xbuf[slot * RB + r, :, cols].astype(F32)
                    y = jnp.concatenate([ys[r, c - 1], ys[r, c]], axis=1)
                    obuf[b % NO, r, :, cols] = (y + res).astype(BF16)

            done = {"u": 0, "d": 0, "s": 0}
            for op in SEQ:
                n, c = divmod(done[op], NT)
                done[op] += 1
                if op == "u":
                    up(n, c)
                elif op == "d":
                    down(rec_rows[n], c, acts[n, c])
                else:
                    down(st_rows[n], c, pltpu.bitcast(hbuf.bitcast(I32)[b * NST + n, c], BF16))
            assert done == {"u": NT * NREC, "d": NT * NREC, "s": NT * NST}
            out_copy(b).start()
            return carry

        jax.lax.fori_loop(0, NB, body, 0)
        for b in range(NB - NO, NB):
            out_copy(b).wait()

    pl.run_scoped(
        pass1,
        pltpu.VMEM((4 * NG, 48, 128), I32),
        pltpu.VMEM((2, NG, 8 * RS, 128), F32),
        pltpu.VMEM((8 * RS + 8, 128), F32),
        pltpu.VMEM((3, 8, 128), F32),
        pltpu.VMEM((4 * NT + 2, C, 128), BF16),
        pltpu.VMEM((E, 128), F32),
        pltpu.VMEM((E, 128), BF16),
    )
    pl.run_scoped(
        pass2,
        pltpu.VMEM((NO, RB, C, W), BF16),
        pltpu.VMEM((NREC * C + C // 2 + 16, W), I32),
        pltpu.VMEM((8 * RS + 8, 128), F32),
        pltpu.VMEM((NREC, 8, 128), F32),
        pltpu.VMEM((C, 128), F32),
        pltpu.VMEM((9 * NG + 1, 8, 128), F32),
    )


@jax.jit
def pallas_standalone__modern_conv_block_convnext_v2__vision_kernel(
    x: jax.Array,
    dw: jax.Array,
    w1: jax.Array,
    w2: jax.Array,
    grn_gamma: jax.Array,
    grn_beta: jax.Array,
):
    B, H, W, C = x.shape
    E = w1.shape[1]
    assert (B, W, C, E) == (1, 512, 96, 384) and dw.shape == (3, 3, C) and H % (2 * U1 * RB) == 0
    hbm = pl.BlockSpec(memory_space=pl.ANY)
    out = pl.pallas_call(
        _kernel,
        out_shape=jax.ShapeDtypeStruct((H, C, W), x.dtype),
        in_specs=[hbm] * 6,
        out_specs=hbm,
        scratch_shapes=[
            pltpu.VMEM((NX * RB, C, W), BF16),
            pltpu.VMEM((H // RB * (RB - NREC), W // 128, E, 128), BF16),
            pltpu.VMEM((E, 128), BF16),
            pltpu.VMEM((C, E), BF16),
            pltpu.VMEM((1, E), F32),
            pltpu.VMEM(dw.shape, BF16),
            pltpu.VMEM((E,), BF16),
            pltpu.VMEM((E,), BF16),
            pltpu.SemaphoreType.DMA((NX,)),
            pltpu.SemaphoreType.DMA((NO,)),
            pltpu.SemaphoreType.DMA((3,)),
        ],
        compiler_params=pltpu.CompilerParams(vmem_limit_bytes=128 * 1024 * 1024, disable_bounds_checks=True),
        name="convnext_v2_block",
    )(jnp.transpose(x, (0, 1, 3, 2)).reshape(H, C, W), dw, w1, w2.T, grn_gamma, grn_beta)
    return jnp.transpose(out.reshape(B, H, C, W), (0, 1, 3, 2))
```

```python
import math

import jax
import jax.numpy as jnp
import jax.experimental.pallas as pl
import jax.experimental.pallas.tpu as pltpu

F32 = jnp.float32
BF16 = jnp.bfloat16
I32 = jnp.int32

RB = 8
NREC = 3
U1 = 2
NX = 4
NO = 2
RS = 9

LAG1 = 5
STATS_AT = 3
SCALE_AT = 4
SEQ = "us" + "usd" * 11 + "sd" + "s" * 7
LAG2 = 5
SIDE_FROM, SIDE_TO = 1, 28
CENTRE_AT = 1
FETCH_AT = 14

_C0 = math.sqrt(2.0 / math.pi)
_K = (_C0 * 0.044715) ** (1.0 / 3.0)
_B = _C0 / _K


def _gelu(z):
    return z * (jnp.tanh(z * (z * z + _B)) + 1.0)


def _ln_scale(var):
    return jax.lax.rsqrt(var + 1e-5) * _K


def _dot(lhs, rhs):
    return jnp.dot(lhs, rhs, preferred_element_type=F32)


def _pad_rows(v):
    return jnp.concatenate([v, jnp.zeros((128 - v.shape[0], v.shape[1]), v.dtype)], axis=0)


def _walsh(a, c):
    p = a & c & 7
    return (1 - 2 * ((p ^ (p >> 1) ^ (p >> 2)) & 1)).astype(F32)


def _tree_sum(parts):
    while len(parts) > 1:
        parts = [parts[i] + parts[i + 1] if i + 1 < len(parts) else parts[i] for i in range(0, len(parts), 2)]
    return parts[0]


def _tiles(v):
    return [v[:, c:c + 128] for c in range(0, v.shape[1], 128)]


def _neighbours(left, right):
    lane = jax.lax.broadcasted_iota(I32, (8, 128), 1)
    zero = jnp.zeros((8, 128), left[0].dtype)
    le = [zero] + [pltpu.roll(v, 1, 1) for v in left]
    ri = [pltpu.roll(v, 127, 1) for v in right] + [zero]
    return ([jnp.where(lane == 0, le[c], le[c + 1]) for c in range(len(left))],
            [jnp.where(lane == 127, ri[c + 1], ri[c]) for c in range(len(right))])


def _kernel(x_hbm, dw_hbm, w1_hbm, w2t_hbm, gamma_hbm, beta_hbm, o_hbm,
            xbuf, hbuf, w1t, wbuf, total, dw_ref, gamma_ref, beta_ref, isem, osem, wsem):
    H, C, W = x_hbm.shape
    E = w1_hbm.shape[1]
    NB = H // RB
    NG = C // 8
    NT = W // 128
    NST = RB - NREC
    rec_rows = list(range(1, 1 + NREC))
    st_rows = [r for r in range(RB) if r not in rec_rows]

    def x_copy(row, n, slot, dst=0):
        return pltpu.make_async_copy(x_hbm.at[pl.ds(row, n)], xbuf.at[pl.ds(slot * RB + dst, n)], isem.at[slot])

    def x_slot(b):
        return (b + U1) % NX

    def block_copy(b):
        return x_copy(b * RB, RB, x_slot(b))

    def tap_columns():
        eye = jax.lax.broadcasted_iota(I32, (C, C), 0) == jax.lax.broadcasted_iota(I32, (C, C), 1)
        rows = [dw_ref[i].astype(F32) for i in range(3)]
        return [jnp.sum(jnp.where(eye, rows[i][j:j + 1, :], 0.0), axis=1, keepdims=True)
                for i in range(3) for j in range(3)]

    def pass1(sbuf, cbuf, rbuf, scale, hnbuf, ssq, w1h):
        R1 = RB * U1
        NI = H // R1
        LAST = R1 - RB + 1
        TAPS = 4 * NT
        hw = hnbuf.bitcast(I32)
        pace = []

        def chunk_copy(t, n=R1):
            return x_copy(t * R1 + RB - 1, n, ((t + 1) % 2) * U1)

        dw_copy = pltpu.make_async_copy(dw_hbm, dw_ref, wsem.at[0])
        w1_copy = pltpu.make_async_copy(w1_hbm, wbuf, wsem.at[1])
        head_copy = x_copy(0, RB - 1, 0, 1)
        late_copies = [pltpu.make_async_copy(w2t_hbm, wbuf, wsem.at[0]),
                       pltpu.make_async_copy(gamma_hbm, gamma_ref, wsem.at[1]),
                       pltpu.make_async_copy(beta_hbm, beta_ref, wsem.at[2])]
        for cp in (dw_copy, w1_copy, head_copy, chunk_copy(0)):
            cp.start()

        dw_copy.wait()
        taps = tap_columns()
        ro = jax.lax.broadcasted_iota(I32, (8, 128), 0)
        co = jax.lax.broadcasted_iota(I32, (8, 128), 1)
        for g in range(NG):
            halves = []
            for o in range(2):
                m = jnp.zeros((8, 128), F32)
                for i in range(3):
                    for j in range(3):
                        m = jnp.where(co == ro + (j * 32 + (i + o) * 8), taps[i * 3 + j][g * 8:(g + 1) * 8], m)
                halves.append(jnp.sum(m, axis=0, keepdims=True) * _walsh(ro, co))
            hnbuf[TAPS + g // 6, 16 * (g % 6):16 * (g % 6) + 16, :] = jnp.concatenate(halves, axis=0).astype(BF16)
        ssq[...] = jnp.zeros_like(ssq)
        xbuf[0] = jnp.zeros((C, W), BF16)

        head_copy.wait()
        w1_copy.wait()
        w1 = wbuf[...]
        w1t[...] = _pad_rows(w1.astype(F32)).T.astype(BF16)
        ra = jax.lax.broadcasted_iota(I32, (128, C), 0)
        ca = jax.lax.broadcasted_iota(I32, (128, C), 1)
        unmix = jnp.where((ra >> 3) == (ca >> 3), _walsh(ra, ca) * 0.125, 0.0).astype(BF16)
        w1h[...] = _dot(unmix, w1).T.astype(BF16)
        for cp in late_copies:
            cp.start()

        def s_at(p, g, j, c):
            return ((p % 2) * NG + g) * 2 + c // 2, pl.ds(8 * (3 * (c % 2) + j), 8)

        def shift(slot, k, g):
            two_rows = xbuf[pl.ds(slot * RB + 2 * k, 2), 8 * g:8 * g + 8, :].reshape(16, W)
            mid = _tiles(pltpu.bitcast(two_rows, I32))
            left, right = _neighbours(mid, mid)
            for j, vs in enumerate((left, mid, right)):
                for c in range(NT):
                    sbuf[s_at(k, g, j, c)] = vs[c]

        def conv(q, g, acc, zero=0):
            rhs = jnp.concatenate([jnp.concatenate([sbuf[s_at(p, g, j, c)] for c in range(NT)], axis=1)
                                   for j in range(3) for p in (q, q + 1)], axis=0)
            lhs = pltpu.bitcast(hw[TAPS + g // 6 + zero, 8 * (g % 6):8 * (g % 6) + 8, :], BF16)
            y = _dot(lhs, _pad_rows(pltpu.bitcast(rhs, BF16)))
            for i, v in enumerate(_tiles(y[0:8]) + _tiles(y[8:16])):
                cbuf[q % 2, g, RS * i:RS * i + 8, :] = v
            pace.append(y[0:8, 0:128])
            acc = y * y if acc is None else acc + y * y
            if g == NG - 1:
                for i, v in enumerate(_tiles(acc[0:8]) + _tiles(acc[8:16])):
                    rbuf[RS * i:RS * i + 8, :] = v
            return acc

        def ln_stats(q):
            sums = [cbuf[q % 2, g, pl.ds(0, 8, stride=RS), :] for g in range(NG)]
            mean8 = _tree_sum(sums) / NG
            centred = [v - mean8 for v in sums]
            for g in range(NG):
                cbuf[q % 2, g, pl.ds(0, 8, stride=RS), :] = centred[g]
            squares = [v * v for v in centred] + [rbuf[pl.ds(k, 8, stride=RS), :] for k in range(1, 8)]
            scale[q % 2] = _ln_scale(_tree_sum(squares) * (0.125 / C))

        def ln_apply(q, i, zero=0):
            if len(pace) >= LAG1:
                scale[2] = pace[-LAG1]
            d = cbuf[q % 2, :, RS * i:RS * i + 8, :] * scale[q % 2 + zero, i:i + 1, :]
            hnbuf[(q % 2) * 2 * NT + i] = d.reshape(C, 128).astype(BF16)

        def up(t, q, g):
            o, e0 = g // (NG // 2), (g % (NG // 2)) * 64
            lhs = pltpu.bitcast(w1h.bitcast(I32)[e0 // 2:e0 // 2 + 32, :], BF16)
            hn = jnp.concatenate([hw[((q % 2) * 2 + o) * NT + c] for c in range(NT)], axis=1)
            a = _gelu(_dot(lhs, _pad_rows(pltpu.bitcast(hn, BF16))))
            ssq[e0:e0 + 64, :] += _tree_sum(_tiles(a * a))
            b, r = divmod(2 * q + o, RB)
            if r in st_rows:
                for c, v in enumerate(_tiles(a)):
                    hbuf[(t * U1 + b) * NST + st_rows.index(r), c, e0:e0 + 64, :] = v.astype(BF16)

        for k in range(2):
            for g in range(NG):
                shift(0, k, g)
        for q in range(2):
            acc = None
            for g in range(NG):
                acc = conv(q, g, acc)
                shift(0, q + 2, g)
            if q == 0:
                ln_stats(0)
                for i in range(2 * NT):
                    ln_apply(0, i)

        def body(t, carry):
            slot = ((t + 1) % 2) * U1
            pl.when(t + 2 < NI)(lambda: chunk_copy(t + 1).start())
            pl.when(t + 2 == NI)(lambda: chunk_copy(NI - 1, LAST).start())
            pl.when(t + 1 < NI)(lambda: chunk_copy(t).wait())

            @pl.when(t + 1 == NI)
            def _():
                chunk_copy(NI - 1, LAST).wait()
                xbuf[slot * RB + LAST] = jnp.zeros((C, W), BF16)
                for b in range(U1):
                    block_copy(b).start()

            zero = t >> 16
            pace.clear()
            for k in range(R1 // 2):
                acc = None
                for g in range(NG):
                    acc = conv(k + 2, g, acc, zero)
                    if g == STATS_AT:
                        ln_stats(k + 1)
                    if g >= SCALE_AT:
                        ln_apply(k + 1, g - SCALE_AT, zero)
                    shift(slot, k, g)
                    up(t, k, g)
            return carry

        jax.lax.fori_loop(0, NI, body, 0)
        for cp in late_copies + [block_copy(0)]:
            cp.wait()
        total[...] = jnp.sum(ssq[...].T, axis=0, keepdims=True)

    def pass2(obuf, cbuf, mean, scale, bias, dwb):
        W2 = NREC * C
        ACC = W2 + C // 2
        for b in range(U1, NX - 1):
            block_copy(b).start()

        def out_copy(b):
            return pltpu.make_async_copy(obuf.at[b % NO], o_hbm.at[pl.ds(b * RB, RB)], osem.at[b % NO])

        inv = 1.0 / (2.0 * _K)
        gx = jnp.sqrt(total[...] * (inv * inv) + 1e-6)
        nx = gx / (jnp.sum(gx, axis=1, keepdims=True) * (1.0 / E) + 1e-6)
        grn = (gamma_ref[...].astype(F32).reshape(1, E) * nx + 1.0) * inv
        for k, col in enumerate(tap_columns()):
            dwb[k * NG:(k + 1) * NG] = jnp.broadcast_to(col, (C, 128)).reshape(NG, 8, 128)
        w2t = wbuf[...].astype(F32)
        cbuf[W2:ACC, 0:E] = pltpu.bitcast((w2t * grn).astype(BF16), I32)
        beta = beta_ref[...].astype(F32).reshape(1, E)
        bias[...] = jnp.broadcast_to(jnp.sum(w2t * beta, axis=1, keepdims=True), (C, 128))

        def conv(slot, n, g, zero=0):
            xs = [xbuf[slot * RB + n + i, 8 * g:8 * g + 8, :].astype(F32) for i in range(3)]
            wt = [jnp.tile(dwb[k * NG + g + (zero if k < 3 else 0)], (1, NT)) for k in range(9)]
            p = [_tiles(xs[0] * wt[j] + xs[1] * wt[3 + j] + xs[2] * wt[6 + j]) for j in range(3)]
            left, right = _neighbours(p[0], p[2])
            y = jnp.concatenate([left[c] + p[1][c] + right[c] for c in range(NT)], axis=1)
            cbuf[n * C + 8 * g:n * C + 8 * g + 8, :] = pltpu.bitcast(y, I32)
            if g > 0:
                y = pltpu.bitcast(cbuf[ACC:ACC + 8, :], F32) + y
            if g < NG - 1:
                cbuf[ACC:ACC + 8, :] = pltpu.bitcast(y, I32)
            else:
                mean[...] = jnp.sum(y, axis=0, keepdims=True) / C

        def centre(n, c):
            rows, cols = slice(n * C, (n + 1) * C), slice(128 * c, 128 * c + 128)
            d = pltpu.bitcast(cbuf[rows, cols], F32) - mean[:, cols]
            cbuf[rows, cols] = pltpu.bitcast(d, I32)
            scale[n, :, cols] = _ln_scale(jnp.sum(d * d, axis=0, keepdims=True) * (1.0 / C))

        side = []
        for i in range(NREC):
            for g in range(NG):
                side.append(("conv", (i + NREC - 1) % NREC, g))
                if CENTRE_AT <= g < CENTRE_AT + NT:
                    side.append(("centre", (i + NREC - 2) % NREC, g - CENTRE_AT))
        cost = [0]
        for kind, _, _ in side:
            cost.append(cost[-1] + (3 if kind == "conv" else 2))
        side_at = [SIDE_FROM + v * (SIDE_TO - SIDE_FROM) // cost[-2] for v in cost[:-1]]
        for n in range(NREC - 1):
            for g in range(NG):
                conv(x_slot(0), n, g)
            if n < NREC - 2:
                for c in range(NT):
                    centre(n, c)

        def body(b, carry):
            pl.when(b + 1 < NB)(lambda: block_copy(b + 1).wait())
            pl.when(b >= NO)(lambda: out_copy(b - NO).wait())
            slot, slot1, zero = x_slot(b), x_slot(b + 1), b >> 16
            acts, ys, pace = {}, {}, []

            def up(n, c):
                y = pltpu.bitcast(cbuf[n * C:(n + 1) * C, 128 * c:128 * c + 128], F32)
                hn = (y * scale[n, :, 128 * c:128 * c + 128]).astype(BF16)
                parts = []
                for k in range(E // C):
                    w = pltpu.bitcast(w1t.bitcast(I32)[C // 2 * k:C // 2 * (k + 1), :], BF16)[:, :C]
                    parts.append(_gelu(_dot(w, hn)))
                acts[n, c] = jnp.concatenate(parts, axis=0).astype(BF16)

            def down(r, c, a):
                i = len(pace)
                if i >= LAG2 and i in side_at:
                    dwb[9 * NG] = pace[-LAG2]
                for at, (kind, n, g) in zip(side_at, side):
                    if at == i and kind == "conv":
                        assert ((n, 0) not in acts) if n == NREC - 1 else ((n, NT - 1) in acts)
                        conv(slot if n == NREC - 1 else slot1, n, g, zero)
                    elif at == i:
                        assert ((n, 0) not in acts) if n >= NREC - 2 else ((n, NT - 1) in acts)
                        centre(n, g)
                if i == FETCH_AT:
                    pl.when(b + NX - 1 < NB)(lambda: block_copy(b + NX - 1).start())
                w = jnp.concatenate([cbuf[pl.ds(pl.multiple_of(W2 + zero * 8, 8), 8), 0:E],
                                     cbuf[W2 + 8:ACC, 0:E]], axis=0)
                ys[r, c] = _dot(pltpu.bitcast(w, BF16), a)
                pace.append(ys[r, c][0:8])
                if c % 2 == 1:
                    cols = slice(128 * c - 128, 128 * c + 128)
                    res = jnp.tile(bias[...], (1, 2)) + xbuf[slot * RB + r, :, cols].astype(F32)
                    y = jnp.concatenate([ys[r, c - 1], ys[r, c]], axis=1)
                    obuf[b % NO, r, :, cols] = (y + res).astype(BF16)

            done = {"u": 0, "d": 0, "s": 0}
            for op in SEQ:
                n, c = divmod(done[op], NT)
                done[op] += 1
                if op == "u":
                    up(n, c)
                elif op == "d":
                    down(rec_rows[n], c, acts[n, c])
                else:
                    down(st_rows[n], c, pltpu.bitcast(hbuf.bitcast(I32)[b * NST + n, c], BF16))
            assert done == {"u": NT * NREC, "d": NT * NREC, "s": NT * NST}
            out_copy(b).start()
            return carry

        jax.lax.fori_loop(0, NB, body, 0)
        for b in range(NB - NO, NB):
            out_copy(b).wait()

    pl.run_scoped(
        pass1,
        pltpu.VMEM((4 * NG, 48, 128), I32),
        pltpu.VMEM((2, NG, 8 * RS, 128), F32),
        pltpu.VMEM((8 * RS + 8, 128), F32),
        pltpu.VMEM((3, 8, 128), F32),
        pltpu.VMEM((4 * NT + 2, C, 128), BF16),
        pltpu.VMEM((E, 128), F32),
        pltpu.VMEM((E, 128), BF16),
    )
    pl.run_scoped(
        pass2,
        pltpu.VMEM((NO, RB, C, W), BF16),
        pltpu.VMEM((NREC * C + C // 2 + 8, W), I32),
        pltpu.VMEM((1, W), F32),
        pltpu.VMEM((NREC, 1, W), F32),
        pltpu.VMEM((C, 128), F32),
        pltpu.VMEM((9 * NG + 1, 8, 128), F32),
    )


@jax.jit
def pallas_standalone__modern_conv_block_convnext_v2__vision_kernel(
    x: jax.Array,
    dw: jax.Array,
    w1: jax.Array,
    w2: jax.Array,
    grn_gamma: jax.Array,
    grn_beta: jax.Array,
):
    B, H, W, C = x.shape
    E = w1.shape[1]
    assert (B, W, C, E) == (1, 512, 96, 384) and dw.shape == (3, 3, C) and H % (2 * U1 * RB) == 0
    hbm = pl.BlockSpec(memory_space=pl.ANY)
    out = pl.pallas_call(
        _kernel,
        out_shape=jax.ShapeDtypeStruct((H, C, W), x.dtype),
        in_specs=[hbm] * 6,
        out_specs=hbm,
        scratch_shapes=[
            pltpu.VMEM((NX * RB, C, W), BF16),
            pltpu.VMEM((H // RB * (RB - NREC), W // 128, E, 128), BF16),
            pltpu.VMEM((E, 128), BF16),
            pltpu.VMEM((C, E), BF16),
            pltpu.VMEM((1, E), F32),
            pltpu.VMEM(dw.shape, BF16),
            pltpu.VMEM((E,), BF16),
            pltpu.VMEM((E,), BF16),
            pltpu.SemaphoreType.DMA((NX,)),
            pltpu.SemaphoreType.DMA((NO,)),
            pltpu.SemaphoreType.DMA((3,)),
        ],
        compiler_params=pltpu.CompilerParams(vmem_limit_bytes=128 * 1024 * 1024, disable_bounds_checks=True),
        name="convnext_v2_block",
    )(jnp.transpose(x, (0, 1, 3, 2)).reshape(H, C, W), dw, w1, w2.T, grn_gamma, grn_beta)
    return jnp.transpose(out.reshape(B, H, C, W), (0, 1, 3, 2))
```

```python
import math

import jax
import jax.numpy as jnp
import jax.experimental.pallas as pl
import jax.experimental.pallas.tpu as pltpu

F32 = jnp.float32
BF16 = jnp.bfloat16
I32 = jnp.int32

RB = 8
NREC = 3
U1 = 2
NX = 4
NO = 2
RS = 9

LAG1 = 4
STATS_AT = 3
SCALE_AT = (4, 5, 6, 7, 8, 9, 10, 11)
NCB = 2
SEQ = "us" + "usd" * 11 + "sd" + "s" * 7
LAG2 = 5
SIDE_FROM, SIDE_TO = 1, 28
CENTRE_AT = (2, 4, 6, 8)
MPACE = 1
FETCH_AT = 14

_C0 = math.sqrt(2.0 / math.pi)
_K = (_C0 * 0.044715) ** (1.0 / 3.0)
_B = _C0 / _K


def _gelu(z):
    return z * (jnp.tanh(z * (z * z + _B)) + 1.0)


def _ln_scale(var):
    return jax.lax.rsqrt(var + 1e-5) * _K


def _dot(lhs, rhs):
    return jnp.dot(lhs, rhs, preferred_element_type=F32)


def _pad_rows(v):
    return jnp.concatenate([v, jnp.zeros((128 - v.shape[0], v.shape[1]), v.dtype)], axis=0)


def _walsh(a, c):
    p = a & c & 7
    return (1 - 2 * ((p ^ (p >> 1) ^ (p >> 2)) & 1)).astype(F32)


def _tree_sum(parts):
    while len(parts) > 1:
        parts = [parts[i] + parts[i + 1] if i + 1 < len(parts) else parts[i] for i in range(0, len(parts), 2)]
    return parts[0]


def _tiles(v):
    return [v[:, c:c + 128] for c in range(0, v.shape[1], 128)]


def _neighbours(left, right):
    lane = jax.lax.broadcasted_iota(I32, (8, 128), 1)
    zero = jnp.zeros((8, 128), left[0].dtype)
    le = [zero] + [pltpu.roll(v, 1, 1) for v in left]
    ri = [pltpu.roll(v, 127, 1) for v in right] + [zero]
    return ([jnp.where(lane == 0, le[c], le[c + 1]) for c in range(len(left))],
            [jnp.where(lane == 127, ri[c + 1], ri[c]) for c in range(len(right))])


def _kernel(x_hbm, dw_hbm, w1_hbm, w2t_hbm, gamma_hbm, beta_hbm, o_hbm,
            xbuf, hbuf, w1t, wbuf, total, dw_ref, gamma_ref, beta_ref, isem, osem, wsem):
    H, C, W = x_hbm.shape
    E = w1_hbm.shape[1]
    NB = H // RB
    NG = C // 8
    NT = W // 128
    NST = RB - NREC
    rec_rows = list(range(1, 1 + NREC))
    st_rows = [r for r in range(RB) if r not in rec_rows]

    def x_copy(row, n, slot, dst=0):
        return pltpu.make_async_copy(x_hbm.at[pl.ds(row, n)], xbuf.at[pl.ds(slot * RB + dst, n)], isem.at[slot])

    def x_slot(b):
        return (b + U1) % NX

    def block_copy(b):
        return x_copy(b * RB, RB, x_slot(b))

    def tap_columns():
        eye = jax.lax.broadcasted_iota(I32, (C, C), 0) == jax.lax.broadcasted_iota(I32, (C, C), 1)
        rows = [dw_ref[i].astype(F32) for i in range(3)]
        return [jnp.sum(jnp.where(eye, rows[i][j:j + 1, :], 0.0), axis=1, keepdims=True)
                for i in range(3) for j in range(3)]

    def pass1(sbuf, rbuf, scale, hnbuf, ssq, w1h, *cbufs):
        R1 = RB * U1
        NI = H // R1
        LAST = R1 - RB + 1
        TAPS = 4 * NT
        hw = hnbuf.bitcast(I32)
        pace = []

        def chunk_copy(t, n=R1):
            return x_copy(t * R1 + RB - 1, n, ((t + 1) % 2) * U1)

        dw_copy = pltpu.make_async_copy(dw_hbm, dw_ref, wsem.at[0])
        w1_copy = pltpu.make_async_copy(w1_hbm, wbuf, wsem.at[1])
        head_copy = x_copy(0, RB - 1, 0, 1)
        late_copies = [pltpu.make_async_copy(w2t_hbm, wbuf, wsem.at[0]),
                       pltpu.make_async_copy(gamma_hbm, gamma_ref, wsem.at[1]),
                       pltpu.make_async_copy(beta_hbm, beta_ref, wsem.at[2])]
        for cp in (dw_copy, w1_copy, head_copy, chunk_copy(0)):
            cp.start()

        dw_copy.wait()
        taps = tap_columns()
        ro = jax.lax.broadcasted_iota(I32, (8, 128), 0)
        co = jax.lax.broadcasted_iota(I32, (8, 128), 1)
        for g in range(NG):
            halves = []
            for o in range(2):
                m = jnp.zeros((8, 128), F32)
                for i in range(3):
                    for j in range(3):
                        m = jnp.where(co == ro + (j * 32 + (i + o) * 8), taps[i * 3 + j][g * 8:(g + 1) * 8], m)
                halves.append(jnp.sum(m, axis=0, keepdims=True) * _walsh(ro, co))
            hnbuf[TAPS + g // 6, 16 * (g % 6):16 * (g % 6) + 16, :] = jnp.concatenate(halves, axis=0).astype(BF16)
        ssq[...] = jnp.zeros_like(ssq)
        xbuf[0] = jnp.zeros((C, W), BF16)

        head_copy.wait()
        w1_copy.wait()
        w1 = wbuf[...]
        w1t[...] = _pad_rows(w1.astype(F32)).T.astype(BF16)
        ra = jax.lax.broadcasted_iota(I32, (128, C), 0)
        ca = jax.lax.broadcasted_iota(I32, (128, C), 1)
        unmix = jnp.where((ra >> 3) == (ca >> 3), _walsh(ra, ca) * 0.125, 0.0).astype(BF16)
        row = jax.lax.broadcasted_iota(I32, (128, E), 0)
        mu = jnp.sum(w1.astype(F32), axis=0, keepdims=True) * (1.0 / C)
        mixed = _dot(unmix, w1) - jnp.where(((row & 7) == 0) & (row < C), mu, 0.0)
        w1h[...] = jnp.where(row == 0, 0.0, mixed).T.astype(BF16)
        for cp in late_copies:
            cp.start()

        def s_at(p, g, j, c):
            return ((p % 2) * NG + g) * 2 + c // 2, pl.ds(8 * (3 * (c % 2) + j), 8)

        def shift(slot, k, g):
            two_rows = xbuf[pl.ds(slot * RB + 2 * k, 2), 8 * g:8 * g + 8, :].reshape(16, W)
            mid = _tiles(pltpu.bitcast(two_rows, I32))
            left, right = _neighbours(mid, mid)
            for j, vs in enumerate((left, mid, right)):
                for c in range(NT):
                    sbuf[s_at(k, g, j, c)] = vs[c]

        def conv(q, g, acc, zero=0):
            rhs = jnp.concatenate([jnp.concatenate([sbuf[s_at(p, g, j, c)] for c in range(NT)], axis=1)
                                   for j in range(3) for p in (q, q + 1)], axis=0)
            lhs = pltpu.bitcast(hw[TAPS + g // 6 + zero, 8 * (g % 6):8 * (g % 6) + 8, :], BF16)
            y = _dot(lhs, _pad_rows(pltpu.bitcast(rhs, BF16)))
            for i, v in enumerate(_tiles(y[0:8]) + _tiles(y[8:16])):
                cbufs[q % NCB][g, RS * i:RS * i + 8, :] = v
            pace.append(y[0:8, 0:128])
            if g == 0:
                return y * y, None, None
            e = cbufs[q % NCB][g, pl.ds(0, 8, stride=RS), :] - cbufs[q % NCB][0, pl.ds(0, 8, stride=RS), :]
            cbufs[q % NCB][g, pl.ds(0, 8, stride=RS), :] = e
            acc = (acc[0] + y * y, e if g == 1 else acc[1] + e, e * e if g == 1 else acc[2] + e * e)
            if g == NG - 1:
                for i, v in enumerate(_tiles(acc[0][0:8]) + _tiles(acc[0][8:16])):
                    rbuf[RS * i:RS * i + 8, :] = v
                rbuf[RS * 8:RS * 8 + 8, :] = acc[2] - acc[1] * acc[1] * (1.0 / NG)
            return acc

        def ln_stats(q, zero=0):
            squares = [rbuf[RS * 8:RS * 8 + 8, :]] + [rbuf[pl.ds(k, 8, stride=RS), :] for k in range(1, 8)]
            scale[q % 2] = _ln_scale(_tree_sum(squares) * (0.125 / C))

        def ln_apply(q, i, zero=0):
            if len(pace) >= LAG1:
                scale[2] = pace[-LAG1]
            d = cbufs[q % NCB][:, RS * i:RS * i + 8, :] * scale[q % 2 + zero, i:i + 1, :]
            hnbuf[(q % 2) * 2 * NT + i] = d.reshape(C, 128).astype(BF16)

        def up(t, q, g):
            o, e0 = g // (NG // 2), (g % (NG // 2)) * 64
            lhs = pltpu.bitcast(w1h.bitcast(I32)[e0 // 2:e0 // 2 + 32, :], BF16)
            hn = jnp.concatenate([hw[((q % 2) * 2 + o) * NT + c] for c in range(NT)], axis=1)
            a = _gelu(_dot(lhs, _pad_rows(pltpu.bitcast(hn, BF16))))
            ssq[e0:e0 + 64, :] += _tree_sum(_tiles(a * a))
            b, r = divmod(2 * q + o, RB)
            if r in st_rows:
                for c, v in enumerate(_tiles(a)):
                    hbuf[(t * U1 + b) * NST + st_rows.index(r), c, e0:e0 + 64, :] = v.astype(BF16)

        for k in range(2):
            for g in range(NG):
                shift(0, k, g)
        for q in range(2):
            acc = None
            for g in range(NG):
                acc = conv(q, g, acc)
                shift(0, q + 2, g)
            if q == 0:
                ln_stats(0)
                for i, at in enumerate(SCALE_AT):
                    if at < NG:
                        ln_apply(0, i)

        def body(t, carry):
            slot = ((t + 1) % 2) * U1
            pl.when(t + 2 < NI)(lambda: chunk_copy(t + 1).start())
            pl.when(t + 2 == NI)(lambda: chunk_copy(NI - 1, LAST).start())
            pl.when(t + 1 < NI)(lambda: chunk_copy(t).wait())

            @pl.when(t + 1 == NI)
            def _():
                chunk_copy(NI - 1, LAST).wait()
                xbuf[slot * RB + LAST] = jnp.zeros((C, W), BF16)
                for b in range(U1):
                    block_copy(b).start()

            zero = t >> 16
            pace.clear()
            for k in range(R1 // 2):
                acc = None
                for g in range(NG):
                    acc = conv(k + 2, g, acc, zero)
                    if g == STATS_AT:
                        ln_stats(k + 1, zero)
                    for i, at in enumerate(SCALE_AT):
                        if at % NG == g:
                            ln_apply(k + 1 - at // NG, i, zero)
                    shift(slot, k, g)
                    up(t, k, g)
            return carry

        jax.lax.fori_loop(0, NI, body, 0)
        for cp in late_copies + [block_copy(0)]:
            cp.wait()
        total[...] = jnp.sum(ssq[...].T, axis=0, keepdims=True)

    def pass2(obuf, cbuf, mean, scale, bias, dwb):
        W2 = NREC * C
        ACC = W2 + C // 2
        for b in range(U1, NX - 1):
            block_copy(b).start()

        def out_copy(b):
            return pltpu.make_async_copy(obuf.at[b % NO], o_hbm.at[pl.ds(b * RB, RB)], osem.at[b % NO])

        inv = 1.0 / (2.0 * _K)
        gx = jnp.sqrt(total[...] * (inv * inv) + 1e-6)
        nx = gx / (jnp.sum(gx, axis=1, keepdims=True) * (1.0 / E) + 1e-6)
        grn = (gamma_ref[...].astype(F32).reshape(1, E) * nx + 1.0) * inv
        for k, col in enumerate(tap_columns()):
            dwb[k * NG:(k + 1) * NG] = jnp.broadcast_to(col, (C, 128)).reshape(NG, 8, 128)
        w2t = wbuf[...].astype(F32)
        cbuf[W2:ACC, 0:E] = pltpu.bitcast((w2t * grn).astype(BF16), I32)
        beta = beta_ref[...].astype(F32).reshape(1, E)
        bias[...] = jnp.broadcast_to(jnp.sum(w2t * beta, axis=1, keepdims=True), (C, 128))

        def conv(slot, n, g, zero=0):
            xs = [xbuf[slot * RB + n + i, 8 * g:8 * g + 8, :].astype(F32) for i in range(3)]
            wt = [jnp.tile(dwb[k * NG + g + (zero if k < 3 else 0)], (1, NT)) for k in range(9)]
            p = [_tiles(xs[0] * wt[j] + xs[1] * wt[3 + j] + xs[2] * wt[6 + j]) for j in range(3)]
            left, right = _neighbours(p[0], p[2])
            y = jnp.concatenate([left[c] + p[1][c] + right[c] for c in range(NT)], axis=1)
            cbuf[n * C + 8 * g:n * C + 8 * g + 8, :] = pltpu.bitcast(y, I32)
            if g > 0:
                y = pltpu.bitcast(cbuf[ACC:ACC + 8, :], F32) + y
            if g < NG - 1:
                cbuf[ACC:ACC + 8, :] = pltpu.bitcast(y, I32)
            else:
                m = jnp.sum(y, axis=0, keepdims=True) / C
                if MPACE:
                    for c, v in enumerate(_tiles(m)):
                        dwb[9 * NG + 1 + c] = jnp.broadcast_to(v, (8, 128))
                else:
                    mean[...] = m

        def centre(n, c, zero=0):
            rows, cols = slice(n * C, (n + 1) * C), slice(128 * c, 128 * c + 128)
            m = jnp.tile(dwb[9 * NG + 1 + c + zero], (NG, 1)) if MPACE else mean[:, cols]
            d = pltpu.bitcast(cbuf[rows, cols], F32) - m
            cbuf[rows, cols] = pltpu.bitcast(d, I32)
            scale[n, :, cols] = _ln_scale(jnp.sum(d * d, axis=0, keepdims=True) * (1.0 / C))

        side = []
        for i in range(NREC):
            for g in range(NG):
                side.append(("conv", (i + NREC - 1) % NREC, g))
                if g in CENTRE_AT:
                    side.append(("centre", (i + NREC - 2) % NREC, CENTRE_AT.index(g)))
        cost = [0]
        for kind, _, _ in side:
            cost.append(cost[-1] + (3 if kind == "conv" else 2))
        side_at = [SIDE_FROM + v * (SIDE_TO - SIDE_FROM) // cost[-2] for v in cost[:-1]]
        for n in range(NREC - 1):
            for g in range(NG):
                conv(x_slot(0), n, g)
            if n < NREC - 2:
                for c in range(NT):
                    centre(n, c)

        def body(b, carry):
            pl.when(b + 1 < NB)(lambda: block_copy(b + 1).wait())
            pl.when(b >= NO)(lambda: out_copy(b - NO).wait())
            slot, slot1, zero = x_slot(b), x_slot(b + 1), b >> 16
            acts, ys, pace = {}, {}, []

            def up(n, c):
                y = pltpu.bitcast(cbuf[n * C:(n + 1) * C, 128 * c:128 * c + 128], F32)
                hn = (y * scale[n, :, 128 * c:128 * c + 128]).astype(BF16)
                parts = []
                for k in range(E // C):
                    w = pltpu.bitcast(w1t.bitcast(I32)[C // 2 * k:C // 2 * (k + 1), :], BF16)[:, :C]
                    parts.append(_gelu(_dot(w, hn)))
                acts[n, c] = jnp.concatenate(parts, axis=0).astype(BF16)

            def down(r, c, a):
                i = len(pace)
                if i >= LAG2 and i in side_at:
                    dwb[9 * NG] = pace[-LAG2]
                for at, (kind, n, g) in zip(side_at, side):
                    if at == i and kind == "conv":
                        assert ((n, 0) not in acts) if n == NREC - 1 else ((n, NT - 1) in acts)
                        conv(slot if n == NREC - 1 else slot1, n, g, zero)
                    elif at == i:
                        assert ((n, g) not in acts) if n >= NREC - 2 else ((n, NT - 1) in acts)
                        centre(n, g, zero)
                if i == FETCH_AT:
                    pl.when(b + NX - 1 < NB)(lambda: block_copy(b + NX - 1).start())
                w = jnp.concatenate([cbuf[pl.ds(pl.multiple_of(W2 + zero * 8, 8), 8), 0:E],
                                     cbuf[W2 + 8:ACC, 0:E]], axis=0)
                ys[r, c] = _dot(pltpu.bitcast(w, BF16), a)
                pace.append(ys[r, c][0:8])
                if c % 2 == 1:
                    cols = slice(128 * c - 128, 128 * c + 128)
                    res = jnp.tile(bias[...], (1, 2)) + xbuf[slot * RB + r, :, cols].astype(F32)
                    y = jnp.concatenate([ys[r, c - 1], ys[r, c]], axis=1)
                    obuf[b % NO, r, :, cols] = (y + res).astype(BF16)

            done = {"u": 0, "d": 0, "s": 0}
            for op in SEQ:
                n, c = divmod(done[op], NT)
                done[op] += 1
                if op == "u":
                    up(n, c)
                elif op == "d":
                    down(rec_rows[n], c, acts[n, c])
                else:
                    down(st_rows[n], c, pltpu.bitcast(hbuf.bitcast(I32)[b * NST + n, c], BF16))
            assert done == {"u": NT * NREC, "d": NT * NREC, "s": NT * NST}
            out_copy(b).start()
            return carry

        jax.lax.fori_loop(0, NB, body, 0)
        for b in range(NB - NO, NB):
            out_copy(b).wait()

    pl.run_scoped(
        pass1,
        pltpu.VMEM((4 * NG, 48, 128), I32),
        pltpu.VMEM((8 * RS + 8, 128), F32),
        pltpu.VMEM((3, 8, 128), F32),
        pltpu.VMEM((4 * NT + 2, C, 128), BF16),
        pltpu.VMEM((E, 128), F32),
        pltpu.VMEM((E, 128), BF16),
        *[pltpu.VMEM((NG, 8 * RS, 128), F32)] * NCB,
    )
    pl.run_scoped(
        pass2,
        pltpu.VMEM((NO, RB, C, W), BF16),
        pltpu.VMEM((NREC * C + C // 2 + 8, W), I32),
        pltpu.VMEM((1, W), F32),
        pltpu.VMEM((NREC, 1, W), F32),
        pltpu.VMEM((C, 128), F32),
        pltpu.VMEM((9 * NG + 1 + NT, 8, 128), F32),
    )


@jax.jit
def pallas_standalone__modern_conv_block_convnext_v2__vision_kernel(
    x: jax.Array,
    dw: jax.Array,
    w1: jax.Array,
    w2: jax.Array,
    grn_gamma: jax.Array,
    grn_beta: jax.Array,
):
    B, H, W, C = x.shape
    E = w1.shape[1]
    assert (B, W, C, E) == (1, 512, 96, 384) and dw.shape == (3, 3, C) and H % (2 * U1 * RB) == 0
    hbm = pl.BlockSpec(memory_space=pl.ANY)
    out = pl.pallas_call(
        _kernel,
        out_shape=jax.ShapeDtypeStruct((H, C, W), x.dtype),
        in_specs=[hbm] * 6,
        out_specs=hbm,
        scratch_shapes=[
            pltpu.VMEM((NX * RB, C, W), BF16),
            pltpu.VMEM((H // RB * (RB - NREC), W // 128, E, 128), BF16),
            pltpu.VMEM((E, 128), BF16),
            pltpu.VMEM((C, E), BF16),
            pltpu.VMEM((1, E), F32),
            pltpu.VMEM(dw.shape, BF16),
            pltpu.VMEM((E,), BF16),
            pltpu.VMEM((E,), BF16),
            pltpu.SemaphoreType.DMA((NX,)),
            pltpu.SemaphoreType.DMA((NO,)),
            pltpu.SemaphoreType.DMA((3,)),
        ],
        compiler_params=pltpu.CompilerParams(vmem_limit_bytes=128 * 1024 * 1024, disable_bounds_checks=True),
        name="convnext_v2_block",
    )(jnp.transpose(x, (0, 1, 3, 2)).reshape(H, C, W), dw, w1, w2.T, grn_gamma, grn_beta)
    return jnp.transpose(out.reshape(B, H, C, W), (0, 1, 3, 2))
```

```python
import math

import jax
import jax.numpy as jnp
import jax.experimental.pallas as pl
import jax.experimental.pallas.tpu as pltpu

F32 = jnp.float32
BF16 = jnp.bfloat16
I32 = jnp.int32

RB = 8
NREC = 3
U1 = 2
NX = 4
NO = 2
RS = 9

LAG1 = 4
STATS_AT = 3
SCALE_AT = (4, 5, 6, 7, 8, 9, 10, 11)
NCB = 2
BATCH = 5
SCN = 4
CC = 2
SEQ = "us" + "usd" * 11 + "sd" + "s" * 7
LAG2 = 5
SIDE_FROM, SIDE_TO = 1, 29
CENTRE_AT = (2, 4, 6, 8)
MPACE = 1
FETCH_AT = 14

_C0 = math.sqrt(2.0 / math.pi)
_K = (_C0 * 0.044715) ** (1.0 / 3.0)
_B = _C0 / _K


def _gelu(z):
    return z * (jnp.tanh(z * (z * z + _B)) + 1.0)


def _ln_scale(var):
    return jax.lax.rsqrt(var + 1e-5) * _K


def _dot(lhs, rhs):
    return jnp.dot(lhs, rhs, preferred_element_type=F32)


def _pad_rows(v):
    return jnp.concatenate([v, jnp.zeros((128 - v.shape[0], v.shape[1]), v.dtype)], axis=0)


def _walsh(a, c):
    p = a & c & 7
    return (1 - 2 * ((p ^ (p >> 1) ^ (p >> 2)) & 1)).astype(F32)


def _tree_sum(parts):
    while len(parts) > 1:
        parts = [parts[i] + parts[i + 1] if i + 1 < len(parts) else parts[i] for i in range(0, len(parts), 2)]
    return parts[0]


def _tiles(v):
    return [v[:, c:c + 128] for c in range(0, v.shape[1], 128)]


def _neighbours(left, right):
    lane = jax.lax.broadcasted_iota(I32, (8, 128), 1)
    zero = jnp.zeros((8, 128), left[0].dtype)
    le = [zero] + [pltpu.roll(v, 1, 1) for v in left]
    ri = [pltpu.roll(v, 127, 1) for v in right] + [zero]
    return ([jnp.where(lane == 0, le[c], le[c + 1]) for c in range(len(left))],
            [jnp.where(lane == 127, ri[c + 1], ri[c]) for c in range(len(right))])


def _kernel(x_hbm, dw_hbm, w1_hbm, w2t_hbm, gamma_hbm, beta_hbm, o_hbm,
            xbuf, hbuf, w1t, wbuf, total, dw_ref, gamma_ref, beta_ref, isem, osem, wsem):
    H, C, W = x_hbm.shape
    E = w1_hbm.shape[1]
    NB = H // RB
    NG = C // 8
    NT = W // 128
    NST = RB - NREC
    rec_rows = list(range(1, 1 + NREC))
    st_rows = [r for r in range(RB) if r not in rec_rows]

    def x_copy(row, n, slot, dst=0):
        return pltpu.make_async_copy(x_hbm.at[pl.ds(row, n)], xbuf.at[pl.ds(slot * RB + dst, n)], isem.at[slot])

    def x_slot(b):
        return (b + U1) % NX

    def block_copy(b):
        return x_copy(b * RB, RB, x_slot(b))

    def tap_columns():
        eye = jax.lax.broadcasted_iota(I32, (C, C), 0) == jax.lax.broadcasted_iota(I32, (C, C), 1)
        rows = [dw_ref[i].astype(F32) for i in range(3)]
        return [jnp.sum(jnp.where(eye, rows[i][j:j + 1, :], 0.0), axis=1, keepdims=True)
                for i in range(3) for j in range(3)]

    def pass1(sbuf, rbuf, scale, hnbuf, ssq, w1h, *cbufs):
        R1 = RB * U1
        NI = H // R1
        LAST = R1 - RB + 1
        TAPS = 4 * NT
        hw = hnbuf.bitcast(I32)
        pace = []

        def chunk_copy(t, n=R1):
            return x_copy(t * R1 + RB - 1, n, ((t + 1) % 2) * U1)

        dw_copy = pltpu.make_async_copy(dw_hbm, dw_ref, wsem.at[0])
        w1_copy = pltpu.make_async_copy(w1_hbm, wbuf, wsem.at[1])
        head_copy = x_copy(0, RB - 1, 0, 1)
        late_copies = [pltpu.make_async_copy(w2t_hbm, wbuf, wsem.at[0]),
                       pltpu.make_async_copy(gamma_hbm, gamma_ref, wsem.at[1]),
                       pltpu.make_async_copy(beta_hbm, beta_ref, wsem.at[2])]
        for cp in (dw_copy, w1_copy, head_copy, chunk_copy(0)):
            cp.start()

        dw_copy.wait()
        taps = tap_columns()
        ro = jax.lax.broadcasted_iota(I32, (8, 128), 0)
        co = jax.lax.broadcasted_iota(I32, (8, 128), 1)
        for g in range(NG):
            halves = []
            for o in range(2):
                m = jnp.zeros((8, 128), F32)
                for i in range(3):
                    for j in range(3):
                        m = jnp.where(co == ro + (j * 32 + (i + o) * 8), taps[i * 3 + j][g * 8:(g + 1) * 8], m)
                halves.append(jnp.sum(m, axis=0, keepdims=True) * _walsh(ro, co))
            hnbuf[TAPS + g // 6, 16 * (g % 6):16 * (g % 6) + 16, :] = jnp.concatenate(halves, axis=0).astype(BF16)
        ssq[...] = jnp.zeros_like(ssq)
        xbuf[0] = jnp.zeros((C, W), BF16)

        head_copy.wait()
        w1_copy.wait()
        w1 = wbuf[...]
        w1t[...] = _pad_rows(w1.astype(F32)).T.astype(BF16)
        ra = jax.lax.broadcasted_iota(I32, (128, C), 0)
        ca = jax.lax.broadcasted_iota(I32, (128, C), 1)
        unmix = jnp.where((ra >> 3) == (ca >> 3), _walsh(ra, ca) * 0.125, 0.0).astype(BF16)
        row = jax.lax.broadcasted_iota(I32, (128, E), 0)
        mu = jnp.sum(w1.astype(F32), axis=0, keepdims=True) * (1.0 / C)
        mixed = _dot(unmix, w1) - jnp.where(((row & 7) == 0) & (row < C), mu, 0.0)
        w1h[...] = jnp.where(row == 0, 0.0, mixed).T.astype(BF16)
        for cp in late_copies:
            cp.start()

        def s_at(p, g, j, c):
            return ((p % 2) * NG + g) * 2 + c // 2, pl.ds(8 * (3 * (c % 2) + j), 8)

        def shift(slot, k, g):
            two_rows = xbuf[pl.ds(slot * RB + 2 * k, 2), 8 * g:8 * g + 8, :].reshape(16, W)
            mid = _tiles(pltpu.bitcast(two_rows, I32))
            left, right = _neighbours(mid, mid)
            for j, vs in enumerate((left, mid, right)):
                for c in range(NT):
                    sbuf[s_at(k, g, j, c)] = vs[c]

        def conv(q, g, acc, zero=0):
            rhs = jnp.concatenate([jnp.concatenate([sbuf[s_at(p, g, j, c)] for c in range(NT)], axis=1)
                                   for j in range(3) for p in (q, q + 1)], axis=0)
            lhs = pltpu.bitcast(hw[TAPS + g // 6 + zero, 8 * (g % 6):8 * (g % 6) + 8, :], BF16)
            y = _dot(lhs, _pad_rows(pltpu.bitcast(rhs, BF16)))
            for i, v in enumerate(_tiles(y[0:8]) + _tiles(y[8:16])):
                cbufs[q % NCB][g, RS * i:RS * i + 8, :] = v
            pace.append(y[0:8, 0:128])
            if g == 0:
                return [y * y]
            acc = [acc[0] + y * y] + acc[1:]
            todo = [(h, zero) for h in range(max(g - BATCH, 1), g)] if g % BATCH == 0 else []
            if g == NG - 1:
                todo += [(h, 0) for h in range(g - g % BATCH, NG)]
            es = [cbufs[q % NCB][h + z, pl.ds(0, 8, stride=RS), :] - cbufs[q % NCB][0, pl.ds(0, 8, stride=RS), :] for h, z in todo]
            for (h, _), e in zip(todo, es):
                cbufs[q % NCB][h, pl.ds(0, 8, stride=RS), :] = e
                acc = [acc[0], e, e * e] if h == 1 else [acc[0], acc[1] + e, acc[2] + e * e]
            if g == NG - 1:
                for i, v in enumerate(_tiles(acc[0][0:8]) + _tiles(acc[0][8:16])):
                    rbuf[RS * i:RS * i + 8, :] = v
                rbuf[RS * 8:RS * 8 + 8, :] = acc[2] - acc[1] * acc[1] * (1.0 / NG)
            return acc

        def ln_stats(q, zero=0):
            squares = [rbuf[RS * 8:RS * 8 + 8, :]] + [rbuf[pl.ds(k, 8, stride=RS), :] for k in range(1, 8)]
            scale[q % 2] = _ln_scale(_tree_sum(squares) * (0.125 / C))

        def ln_apply(q, i, zero=0):
            if len(pace) >= LAG1:
                scale[2] = pace[-LAG1]
            d = cbufs[q % NCB][:, RS * i:RS * i + 8, :] * scale[q % 2 + zero, i:i + 1, :]
            hnbuf[(q % 2) * 2 * NT + i] = d.reshape(C, 128).astype(BF16)

        def up(t, q, g):
            o, e0 = g // (NG // 2), (g % (NG // 2)) * 64
            lhs = pltpu.bitcast(w1h.bitcast(I32)[e0 // 2:e0 // 2 + 32, :], BF16)
            hn = jnp.concatenate([hw[((q % 2) * 2 + o) * NT + c] for c in range(NT)], axis=1)
            a = _gelu(_dot(lhs, _pad_rows(pltpu.bitcast(hn, BF16))))
            ssq[e0:e0 + 64, :] += _tree_sum(_tiles(a * a))
            b, r = divmod(2 * q + o, RB)
            if r in st_rows:
                for c, v in enumerate(_tiles(a)):
                    hbuf[(t * U1 + b) * NST + st_rows.index(r), c, e0:e0 + 64, :] = v.astype(BF16)

        for k in range(2):
            for g in range(NG):
                shift(0, k, g)
        for q in range(2):
            acc = None
            for g in range(NG):
                acc = conv(q, g, acc)
                shift(0, q + 2, g)
            if q == 0:
                ln_stats(0)
                for i, at in enumerate(SCALE_AT):
                    if at < NG:
                        ln_apply(0, i)

        def body(t, carry):
            slot = ((t + 1) % 2) * U1
            pl.when(t + 2 < NI)(lambda: chunk_copy(t + 1).start())
            pl.when(t + 2 == NI)(lambda: chunk_copy(NI - 1, LAST).start())
            pl.when(t + 1 < NI)(lambda: chunk_copy(t).wait())

            @pl.when(t + 1 == NI)
            def _():
                chunk_copy(NI - 1, LAST).wait()
                xbuf[slot * RB + LAST] = jnp.zeros((C, W), BF16)
                for b in range(U1):
                    block_copy(b).start()

            zero = t >> 16
            pace.clear()
            for k in range(R1 // 2):
                acc = None
                for g in range(NG):
                    acc = conv(k + 2, g, acc, zero)
                    if g == STATS_AT:
                        ln_stats(k + 1, zero)
                    for i, at in enumerate(SCALE_AT):
                        if at % NG == g:
                            ln_apply(k + 1 - at // NG, i, zero)
                    shift(slot, k, g)
                    up(t, k, g)
            return carry

        jax.lax.fori_loop(0, NI, body, 0)
        for cp in late_copies + [block_copy(0)]:
            cp.wait()
        total[0] = jnp.sum(ssq[...].T, axis=0, keepdims=True)

    def pass2(obuf, cbuf, mean, scale, bias, dwb):
        W2 = NREC * C
        ACC = W2 + C // 2
        for b in range(U1, NX - 1):
            block_copy(b).start()

        def out_copy(b):
            return pltpu.make_async_copy(obuf.at[b % NO], o_hbm.at[pl.ds(b * RB, RB)], osem.at[b % NO])

        inv = 1.0 / (2.0 * _K)
        gx = jnp.sqrt(total[0] * (inv * inv) + 1e-6)
        nx = gx / (jnp.sum(gx, axis=1, keepdims=True) * (1.0 / E) + 1e-6)
        grn = (gamma_ref[...].astype(F32).reshape(1, E) * nx + 1.0) * inv
        for k, col in enumerate(tap_columns()):
            dwb[k * NG:(k + 1) * NG] = jnp.broadcast_to(col, (C, 128)).reshape(NG, 8, 128)
        w2t = wbuf[...].astype(F32)
        cbuf[W2:ACC, 0:E] = pltpu.bitcast((w2t * grn).astype(BF16), I32)
        beta = beta_ref[...].astype(F32).reshape(1, E)
        bias[...] = jnp.broadcast_to(jnp.sum(w2t * beta, axis=1, keepdims=True), (C, 128))

        def conv(slot, n, g, zero=0):
            xs = [xbuf[slot * RB + n + i, 8 * g:8 * g + 8, :].astype(F32) for i in range(3)]
            wt = [jnp.tile(dwb[k * NG + g + (zero if k < 3 else 0)], (1, NT)) for k in range(9)]
            p = [_tiles(xs[0] * wt[j] + xs[1] * wt[3 + j] + xs[2] * wt[6 + j]) for j in range(3)]
            left, right = _neighbours(p[0], p[2])
            y = jnp.concatenate([left[c] + p[1][c] + right[c] for c in range(NT)], axis=1)
            cbuf[n * C + 8 * g:n * C + 8 * g + 8, :] = pltpu.bitcast(y, I32)
            if g > 0:
                y = pltpu.bitcast(cbuf[ACC:ACC + 8, :], F32) + y
            if g < NG - 1:
                cbuf[ACC:ACC + 8, :] = pltpu.bitcast(y, I32)
            else:
                m = jnp.sum(y, axis=0, keepdims=True) / C
                if MPACE:
                    for c, v in enumerate(_tiles(m)):
                        dwb[9 * NG + 1 + c] = jnp.broadcast_to(v, (8, 128))
                else:
                    mean[...] = m

        def centre(n, c, zero=0):
            rows, cols = slice(n * C, (n + 1) * C), slice(128 * c, 128 * c + 128)
            m = jnp.tile(dwb[9 * NG + 1 + c + zero], (NG, 1)) if MPACE else mean[:, cols]
            d = pltpu.bitcast(cbuf[rows, cols], F32) - m
            cbuf[rows, cols] = pltpu.bitcast(d, I32)
            scale[n, :, cols] = _ln_scale(jnp.sum(d * d, axis=0, keepdims=True) * (1.0 / C))

        side = []
        for i in range(NREC):
            for g in range(NG):
                side.append(("conv", (i + NREC - 1) % NREC, g))
                if g in CENTRE_AT:
                    side.append(("centre", (i + NREC - 2) % NREC, CENTRE_AT.index(g)))
        cost = [0]
        for kind, _, _ in side:
            cost.append(cost[-1] + (3 if kind == "conv" else CC))
        side_at = [SIDE_FROM + v * (SIDE_TO - SIDE_FROM) // cost[-2] for v in cost[:-1]]
        for n in range(NREC - 1):
            for g in range(NG):
                conv(x_slot(0), n, g)
            if n < NREC - 2:
                for c in range(NT):
                    centre(n, c)

        def body(b, carry):
            pl.when(b + 1 < NB)(lambda: block_copy(b + 1).wait())
            pl.when(b >= NO)(lambda: out_copy(b - NO).wait())
            slot, slot1, zero = x_slot(b), x_slot(b + 1), b >> 16
            acts, ys, pace = {}, {}, []

            def up(n, c):
                y = pltpu.bitcast(cbuf[n * C:(n + 1) * C, 128 * c:128 * c + 128], F32)
                hn = (y * scale[n, :, 128 * c:128 * c + 128]).astype(BF16)
                parts = []
                for k in range(E // C):
                    w = pltpu.bitcast(w1t.bitcast(I32)[C // 2 * k:C // 2 * (k + 1), :], BF16)[:, :C]
                    parts.append(_gelu(_dot(w, hn)))
                acts[n, c] = jnp.concatenate(parts, axis=0).astype(BF16)

            def down(r, c, a):
                i = len(pace)
                if i >= LAG2 and i in side_at:
                    dwb[9 * NG] = pace[-LAG2]
                for at, (kind, n, g) in zip(side_at, side):
                    if at == i and kind == "conv":
                        assert ((n, 0) not in acts) if n == NREC - 1 else ((n, NT - 1) in acts)
                        conv(slot if n == NREC - 1 else slot1, n, g, zero)
                    elif at == i:
                        assert ((n, g) not in acts) if n >= NREC - 2 else ((n, NT - 1) in acts)
                        centre(n, g, zero)
                if i == FETCH_AT:
                    pl.when(b + NX - 1 < NB)(lambda: block_copy(b + NX - 1).start())
                w = jnp.concatenate([cbuf[pl.ds(pl.multiple_of(W2 + zero * 8, 8), 8), 0:E],
                                     cbuf[W2 + 8:ACC, 0:E]], axis=0)
                ys[r, c] = _dot(pltpu.bitcast(w, BF16), a)
                pace.append(ys[r, c][0:8])
                if c % 2 == 1:
                    cols = slice(128 * c - 128, 128 * c + 128)
                    res = jnp.tile(bias[...], (1, 2)) + xbuf[slot * RB + r, :, cols].astype(F32)
                    y = jnp.concatenate([ys[r, c - 1], ys[r, c]], axis=1)
                    obuf[b % NO, r, :, cols] = (y + res).astype(BF16)

            done = {"u": 0, "d": 0, "s": 0}
            for op in SEQ:
                n, c = divmod(done[op], NT)
                done[op] += 1
                if op == "u":
                    up(n, c)
                elif op == "d":
                    down(rec_rows[n], c, acts[n, c])
                else:
                    down(st_rows[n], c, pltpu.bitcast(hbuf.bitcast(I32)[b * NST + n, c], BF16))
            assert done == {"u": NT * NREC, "d": NT * NREC, "s": NT * NST}
            out_copy(b).start()
            return carry

        jax.lax.fori_loop(0, NB, body, 0)
        for b in range(NB - NO, NB):
            out_copy(b).wait()

    pl.run_scoped(
        pass1,
        pltpu.VMEM((4 * NG, 48, 128), I32),
        pltpu.VMEM((8 * RS + 8, 128), F32),
        pltpu.VMEM((3, 8, 128), F32),
        pltpu.VMEM((4 * NT + 2, C, 128), BF16),
        pltpu.VMEM((E, 128), F32),
        pltpu.VMEM((E, 128), BF16),
        *[pltpu.VMEM((NG, 8 * RS, 128), F32)] * NCB,
    )
    pl.run_scoped(
        pass2,
        pltpu.VMEM((NO, RB, C, W), BF16),
        pltpu.VMEM((NREC * C + C // 2 + 8, W), I32),
        pltpu.VMEM((1, W), F32),
        pltpu.VMEM((SCN, 1, W), F32),
        pltpu.VMEM((C, 128), F32),
        pltpu.VMEM((9 * NG + 1 + NT, 8, 128), F32),
    )


@jax.jit
def pallas_standalone__modern_conv_block_convnext_v2__vision_kernel(
    x: jax.Array,
    dw: jax.Array,
    w1: jax.Array,
    w2: jax.Array,
    grn_gamma: jax.Array,
    grn_beta: jax.Array,
):
    B, H, W, C = x.shape
    E = w1.shape[1]
    assert (B, W, C, E) == (1, 512, 96, 384) and dw.shape == (3, 3, C) and H % (2 * U1 * RB) == 0
    hbm = pl.BlockSpec(memory_space=pl.ANY)
    out = pl.pallas_call(
        _kernel,
        out_shape=jax.ShapeDtypeStruct((H, C, W), x.dtype),
        in_specs=[hbm] * 6,
        out_specs=hbm,
        scratch_shapes=[
            pltpu.VMEM((NX * RB, C, W), BF16),
            pltpu.VMEM((H // RB * (RB - NREC), W // 128, E, 128), BF16),
            pltpu.VMEM((E, 128), BF16),
            pltpu.VMEM((C, E), BF16),
            pltpu.VMEM((2, 1, E), F32),
            pltpu.VMEM(dw.shape, BF16),
            pltpu.VMEM((E,), BF16),
            pltpu.VMEM((E,), BF16),
            pltpu.SemaphoreType.DMA((NX,)),
            pltpu.SemaphoreType.DMA((NO,)),
            pltpu.SemaphoreType.DMA((3,)),
        ],
        compiler_params=pltpu.CompilerParams(vmem_limit_bytes=128 * 1024 * 1024, disable_bounds_checks=True),
        name="convnext_v2_block",
    )(jnp.transpose(x, (0, 1, 3, 2)).reshape(H, C, W), dw, w1, w2.T, grn_gamma, grn_beta)
    return jnp.transpose(out.reshape(B, H, C, W), (0, 1, 3, 2))
```

```python
import math

import jax
import jax.numpy as jnp
import jax.experimental.pallas as pl
import jax.experimental.pallas.tpu as pltpu

F32 = jnp.float32
BF16 = jnp.bfloat16
I32 = jnp.int32

RB = 8
NREC = 3
U1 = 2
NX = 4
NO = 2
RS = 9

LAG1 = 4
STATS_AT = 3
PIVOT_EVERY = 5
SEQ = "us" + "usd" * 11 + "ssd" + "s" * 6
LAG2 = 5
SIDE_FROM, SIDE_TO = 1, 29
CENTRE_AT = (2, 4, 6, 8)
FETCH_AT = 14

_C0 = math.sqrt(2.0 / math.pi)
_K = (_C0 * 0.044715) ** (1.0 / 3.0)
_B = _C0 / _K


def _gelu(z):
    return z * (jnp.tanh(z * (z * z + _B)) + 1.0)


def _ln_scale(var):
    return jax.lax.rsqrt(var + 1e-5) * _K


def _dot(lhs, rhs):
    return jnp.dot(lhs, rhs, preferred_element_type=F32)


def _pad_rows(v):
    return jnp.concatenate([v, jnp.zeros((128 - v.shape[0], v.shape[1]), v.dtype)], axis=0)


def _walsh(a, c):
    p = a & c & 7
    return (1 - 2 * ((p ^ (p >> 1) ^ (p >> 2)) & 1)).astype(F32)


def _tree_sum(parts):
    while len(parts) > 1:
        parts = [parts[i] + parts[i + 1] if i + 1 < len(parts) else parts[i] for i in range(0, len(parts), 2)]
    return parts[0]


def _tiles(v):
    return [v[:, c:c + 128] for c in range(0, v.shape[1], 128)]


def _neighbours(left, right):
    lane = jax.lax.broadcasted_iota(I32, (8, 128), 1)
    zero = jnp.zeros((8, 128), left[0].dtype)
    le = [zero] + [pltpu.roll(v, 1, 1) for v in left]
    ri = [pltpu.roll(v, 127, 1) for v in right] + [zero]
    return ([jnp.where(lane == 0, le[c], le[c + 1]) for c in range(len(left))],
            [jnp.where(lane == 127, ri[c + 1], ri[c]) for c in range(len(right))])


def _kernel(x_hbm, dw_hbm, w1_hbm, w2t_hbm, gamma_hbm, beta_hbm, o_hbm,
            xbuf, hbuf, w1t, wbuf, total, dw_ref, gamma_ref, beta_ref, isem, osem, wsem):
    H, C, W = x_hbm.shape
    E = w1_hbm.shape[1]
    NB = H // RB
    NG = C // 8
    NT = W // 128
    NST = RB - NREC
    rec_rows = list(range(1, 1 + NREC))
    st_rows = [r for r in range(RB) if r not in rec_rows]

    def x_copy(row, n, slot, dst=0):
        return pltpu.make_async_copy(x_hbm.at[pl.ds(row, n)], xbuf.at[pl.ds(slot * RB + dst, n)], isem.at[slot])

    def x_slot(b):
        return (b + U1) % NX

    def block_copy(b):
        return x_copy(b * RB, RB, x_slot(b))

    def tap_columns():
        eye = jax.lax.broadcasted_iota(I32, (C, C), 0) == jax.lax.broadcasted_iota(I32, (C, C), 1)
        rows = [dw_ref[i].astype(F32) for i in range(3)]
        return [jnp.sum(jnp.where(eye, rows[i][j:j + 1, :], 0.0), axis=1, keepdims=True)
                for i in range(3) for j in range(3)]

    def pass1(sbuf, rbuf, scale, hnbuf, ssq, w1h, *cbufs):
        R1 = RB * U1
        NI = H // R1
        LAST = R1 - RB + 1
        TAPS = 4 * NT
        hw = hnbuf.bitcast(I32)
        pace = []

        def chunk_copy(t, n=R1):
            return x_copy(t * R1 + RB - 1, n, ((t + 1) % 2) * U1)

        dw_copy = pltpu.make_async_copy(dw_hbm, dw_ref, wsem.at[0])
        w1_copy = pltpu.make_async_copy(w1_hbm, wbuf, wsem.at[1])
        head_copy = x_copy(0, RB - 1, 0, 1)
        late_copies = [pltpu.make_async_copy(w2t_hbm, wbuf, wsem.at[0]),
                       pltpu.make_async_copy(gamma_hbm, gamma_ref, wsem.at[1]),
                       pltpu.make_async_copy(beta_hbm, beta_ref, wsem.at[2])]
        for cp in (dw_copy, w1_copy, head_copy, chunk_copy(0)):
            cp.start()

        dw_copy.wait()
        taps = tap_columns()
        ro = jax.lax.broadcasted_iota(I32, (8, 128), 0)
        co = jax.lax.broadcasted_iota(I32, (8, 128), 1)
        for g in range(NG):
            halves = []
            for o in range(2):
                m = jnp.zeros((8, 128), F32)
                for i in range(3):
                    for j in range(3):
                        m = jnp.where(co == ro + (j * 32 + (i + o) * 8), taps[i * 3 + j][g * 8:(g + 1) * 8], m)
                halves.append(jnp.sum(m, axis=0, keepdims=True) * _walsh(ro, co))
            hnbuf[TAPS + g // 6, 16 * (g % 6):16 * (g % 6) + 16, :] = jnp.concatenate(halves, axis=0).astype(BF16)
        ssq[...] = jnp.zeros_like(ssq)
        xbuf[0] = jnp.zeros((C, W), BF16)

        head_copy.wait()
        w1_copy.wait()
        w1 = wbuf[...]
        w1t[...] = _pad_rows(w1.astype(F32)).T.astype(BF16)
        ra = jax.lax.broadcasted_iota(I32, (128, C), 0)
        ca = jax.lax.broadcasted_iota(I32, (128, C), 1)
        unmix = jnp.where((ra >> 3) == (ca >> 3), _walsh(ra, ca) * 0.125, 0.0).astype(BF16)
        row = jax.lax.broadcasted_iota(I32, (128, E), 0)
        mu = jnp.sum(w1.astype(F32), axis=0, keepdims=True) * (1.0 / C)
        mixed = _dot(unmix, w1) - jnp.where(((row & 7) == 0) & (row < C), mu, 0.0)
        w1h[...] = jnp.where(row == 0, 0.0, mixed).T.astype(BF16)
        for cp in late_copies:
            cp.start()

        def s_at(p, g, j, c):
            return ((p % 2) * NG + g) * 2 + c // 2, pl.ds(8 * (3 * (c % 2) + j), 8)

        def shift(slot, k, g):
            two_rows = xbuf[pl.ds(slot * RB + 2 * k, 2), 8 * g:8 * g + 8, :].reshape(16, W)
            mid = _tiles(pltpu.bitcast(two_rows, I32))
            left, right = _neighbours(mid, mid)
            for j, vs in enumerate((left, mid, right)):
                for c in range(NT):
                    sbuf[s_at(k, g, j, c)] = vs[c]

        def conv(q, g, acc, zero=0):
            rhs = jnp.concatenate([jnp.concatenate([sbuf[s_at(p, g, j, c)] for c in range(NT)], axis=1)
                                   for j in range(3) for p in (q, q + 1)], axis=0)
            lhs = pltpu.bitcast(hw[TAPS + g // 6 + zero, 8 * (g % 6):8 * (g % 6) + 8, :], BF16)
            y = _dot(lhs, _pad_rows(pltpu.bitcast(rhs, BF16)))
            for i, v in enumerate(_tiles(y[0:8]) + _tiles(y[8:16])):
                cbufs[q % 2][g, RS * i:RS * i + 8, :] = v
            pace.append(y[0:8, 0:128])
            if g == 0:
                return [y * y]
            acc = [acc[0] + y * y] + acc[1:]
            todo = [(h, zero) for h in range(max(g - PIVOT_EVERY, 1), g)] if g % PIVOT_EVERY == 0 else []
            if g == NG - 1:
                todo += [(h, 0) for h in range(g - g % PIVOT_EVERY, NG)]
            first = pl.ds(0, 8, stride=RS)
            es = [cbufs[q % 2][h + z, first, :] - cbufs[q % 2][0, first, :] for h, z in todo]
            for (h, _), e in zip(todo, es):
                cbufs[q % 2][h, first, :] = e
                acc = [acc[0], e, e * e] if h == 1 else [acc[0], acc[1] + e, acc[2] + e * e]
            if g == NG - 1:
                for i, v in enumerate(_tiles(acc[0][0:8]) + _tiles(acc[0][8:16])):
                    rbuf[RS * i:RS * i + 8, :] = v
                rbuf[RS * 8:RS * 8 + 8, :] = acc[2] - acc[1] * acc[1] * (1.0 / NG)
            return acc

        def ln_stats(q):
            squares = [rbuf[RS * 8:RS * 8 + 8, :]] + [rbuf[pl.ds(k, 8, stride=RS), :] for k in range(1, 8)]
            scale[q % 2] = _ln_scale(_tree_sum(squares) * (0.125 / C))

        def ln_apply(q, i, zero=0):
            if len(pace) >= LAG1:
                scale[2] = pace[-LAG1]
            d = cbufs[q % 2][:, RS * i:RS * i + 8, :] * scale[q % 2 + zero, i:i + 1, :]
            hnbuf[(q % 2) * 2 * NT + i] = d.reshape(C, 128).astype(BF16)

        def up(t, q, g):
            o, e0 = g // (NG // 2), (g % (NG // 2)) * 64
            lhs = pltpu.bitcast(w1h.bitcast(I32)[e0 // 2:e0 // 2 + 32, :], BF16)
            hn = jnp.concatenate([hw[((q % 2) * 2 + o) * NT + c] for c in range(NT)], axis=1)
            a = _gelu(_dot(lhs, _pad_rows(pltpu.bitcast(hn, BF16))))
            ssq[e0:e0 + 64, :] += _tree_sum(_tiles(a * a))
            b, r = divmod(2 * q + o, RB)
            if r in st_rows:
                for c, v in enumerate(_tiles(a)):
                    hbuf[(t * U1 + b) * NST + st_rows.index(r), c, e0:e0 + 64, :] = v.astype(BF16)

        for k in range(2):
            for g in range(NG):
                shift(0, k, g)
        for q in range(2):
            acc = None
            for g in range(NG):
                acc = conv(q, g, acc)
                shift(0, q + 2, g)
            if q == 0:
                ln_stats(0)
                for i in range(2 * NT):
                    ln_apply(0, i)

        def body(t, carry):
            slot = ((t + 1) % 2) * U1
            pl.when(t + 1 < NI)(lambda: chunk_copy(t).wait())

            @pl.when(t + 1 == NI)
            def _():
                chunk_copy(NI - 1, LAST).wait()
                xbuf[slot * RB + LAST] = jnp.zeros((C, W), BF16)
                for b in range(U1):
                    block_copy(b).start()

            zero = t >> 16
            pace.clear()
            for k in range(R1 // 2):
                acc = None
                for g in range(NG):
                    acc = conv(k + 2, g, acc, zero)
                    if g == STATS_AT:
                        ln_stats(k + 1)
                    if g > STATS_AT:
                        ln_apply(k + 1, g - STATS_AT - 1, zero)
                    if (k, g) == (0, 0):
                        pl.when(t + 2 < NI)(lambda: chunk_copy(t + 1).start())
                        pl.when(t + 2 == NI)(lambda: chunk_copy(NI - 1, LAST).start())
                    shift(slot, k, g)
                    up(t, k, g)
            return carry

        jax.lax.fori_loop(0, NI, body, 0)
        for cp in late_copies + [block_copy(0)]:
            cp.wait()
        total[0] = jnp.sum(ssq[...].T, axis=0, keepdims=True)

    def pass2(obuf, cbuf, scale, bias, dwb):
        W2 = NREC * C
        ACC = W2 + C // 2
        MEAN = 9 * NG + 1
        for b in range(U1, NX - 1):
            block_copy(b).start()

        def out_copy(b):
            return pltpu.make_async_copy(obuf.at[b % NO], o_hbm.at[pl.ds(b * RB, RB)], osem.at[b % NO])

        inv = 1.0 / (2.0 * _K)
        gx = jnp.sqrt(total[0] * (inv * inv) + 1e-6)
        nx = gx / (jnp.sum(gx, axis=1, keepdims=True) * (1.0 / E) + 1e-6)
        grn = (gamma_ref[...].astype(F32).reshape(1, E) * nx + 1.0) * inv
        for k, col in enumerate(tap_columns()):
            dwb[k * NG:(k + 1) * NG] = jnp.broadcast_to(col, (C, 128)).reshape(NG, 8, 128)
        w2t = wbuf[...].astype(F32)
        cbuf[W2:ACC, 0:E] = pltpu.bitcast((w2t * grn).astype(BF16), I32)
        beta = beta_ref[...].astype(F32).reshape(1, E)
        bias[...] = jnp.broadcast_to(jnp.sum(w2t * beta, axis=1, keepdims=True), (C, 128))

        def conv(slot, n, g, zero=0):
            xs = [xbuf[slot * RB + n + i, 8 * g:8 * g + 8, :].astype(F32) for i in range(3)]
            wt = [jnp.tile(dwb[k * NG + g + (zero if k < 3 else 0)], (1, NT)) for k in range(9)]
            p = [_tiles(xs[0] * wt[j] + xs[1] * wt[3 + j] + xs[2] * wt[6 + j]) for j in range(3)]
            left, right = _neighbours(p[0], p[2])
            y = jnp.concatenate([left[c] + p[1][c] + right[c] for c in range(NT)], axis=1)
            cbuf[n * C + 8 * g:n * C + 8 * g + 8, :] = pltpu.bitcast(y, I32)
            if g > 0:
                y = pltpu.bitcast(cbuf[ACC:ACC + 8, :], F32) + y
            if g < NG - 1:
                cbuf[ACC:ACC + 8, :] = pltpu.bitcast(y, I32)
            else:
                for c, v in enumerate(_tiles(jnp.sum(y, axis=0, keepdims=True) / C)):
                    dwb[MEAN + c] = jnp.broadcast_to(v, (8, 128))

        def centre(n, c, zero=0):
            rows, cols = slice(n * C, (n + 1) * C), slice(128 * c, 128 * c + 128)
            d = pltpu.bitcast(cbuf[rows, cols], F32) - jnp.tile(dwb[MEAN + c + zero], (NG, 1))
            cbuf[rows, cols] = pltpu.bitcast(d, I32)
            scale[n, :, cols] = _ln_scale(jnp.sum(d * d, axis=0, keepdims=True) * (1.0 / C))

        side = []
        for i in range(NREC):
            for g in range(NG):
                side.append(("conv", (i + NREC - 1) % NREC, g))
                if g in CENTRE_AT:
                    side.append(("centre", (i + NREC - 2) % NREC, CENTRE_AT.index(g)))
        cost = [0]
        for kind, _, _ in side:
            cost.append(cost[-1] + (3 if kind == "conv" else 1))
        side_at = [SIDE_FROM + v * (SIDE_TO - SIDE_FROM) // cost[-2] for v in cost[:-1]]
        for n in range(NREC - 1):
            for g in range(NG):
                conv(x_slot(0), n, g)
            if n < NREC - 2:
                for c in range(NT):
                    centre(n, c)

        def body(b, carry):
            pl.when(b + 1 < NB)(lambda: block_copy(b + 1).wait())
            pl.when(b >= NO)(lambda: out_copy(b - NO).wait())
            slot, slot1, zero = x_slot(b), x_slot(b + 1), b >> 16
            acts, ys, pace = {}, {}, []

            def up(n, c):
                y = pltpu.bitcast(cbuf[n * C:(n + 1) * C, 128 * c:128 * c + 128], F32)
                hn = (y * scale[n, :, 128 * c:128 * c + 128]).astype(BF16)
                parts = []
                for k in range(E // C):
                    w = pltpu.bitcast(w1t.bitcast(I32)[C // 2 * k:C // 2 * (k + 1), :], BF16)[:, :C]
                    parts.append(_gelu(_dot(w, hn)))
                acts[n, c] = jnp.concatenate(parts, axis=0).astype(BF16)

            def down(r, c, a):
                i = len(pace)
                if i >= LAG2 and i in side_at:
                    dwb[9 * NG] = pace[-LAG2]
                for at, (kind, n, g) in zip(side_at, side):
                    if at == i and kind == "conv":
                        assert ((n, 0) not in acts) if n == NREC - 1 else ((n, NT - 1) in acts)
                        conv(slot if n == NREC - 1 else slot1, n, g, zero)
                    elif at == i:
                        assert ((n, g) not in acts) if n >= NREC - 2 else ((n, NT - 1) in acts)
                        centre(n, g, zero)
                if i == FETCH_AT:
                    pl.when(b + NX - 1 < NB)(lambda: block_copy(b + NX - 1).start())
                w = jnp.concatenate([cbuf[pl.ds(pl.multiple_of(W2 + zero * 8, 8), 8), 0:E],
                                     cbuf[W2 + 8:ACC, 0:E]], axis=0)
                ys[r, c] = _dot(pltpu.bitcast(w, BF16), a)
                pace.append(ys[r, c][0:8])
                if c % 2 == 1:
                    cols = slice(128 * c - 128, 128 * c + 128)
                    res = jnp.tile(bias[...], (1, 2)) + xbuf[slot * RB + r, :, cols].astype(F32)
                    y = jnp.concatenate([ys[r, c - 1], ys[r, c]], axis=1)
                    obuf[b % NO, r, :, cols] = (y + res).astype(BF16)

            done = {"u": 0, "d": 0, "s": 0}
            for op in SEQ:
                n, c = divmod(done[op], NT)
                done[op] += 1
                if op == "u":
                    up(n, c)
                elif op == "d":
                    down(rec_rows[n], c, acts[n, c])
                else:
                    down(st_rows[n], c, pltpu.bitcast(hbuf.bitcast(I32)[b * NST + n, c], BF16))
            assert done == {"u": NT * NREC, "d": NT * NREC, "s": NT * NST}
            out_copy(b).start()
            return carry

        jax.lax.fori_loop(0, NB, body, 0)
        for b in range(NB - NO, NB):
            out_copy(b).wait()

    pl.run_scoped(
        pass1,
        pltpu.VMEM((4 * NG, 48, 128), I32),
        pltpu.VMEM((8 * RS + 8, 128), F32),
        pltpu.VMEM((3, 8, 128), F32),
        pltpu.VMEM((4 * NT + 2, C, 128), BF16),
        pltpu.VMEM((E, 128), F32),
        pltpu.VMEM((E, 128), BF16),
        *[pltpu.VMEM((NG, 8 * RS, 128), F32)] * 2,
    )
    pl.run_scoped(
        pass2,
        pltpu.VMEM((NO, RB, C, W), BF16),
        pltpu.VMEM((NREC * C + C // 2 + 8, W), I32),
        pltpu.VMEM((NREC + 1, 1, W), F32),
        pltpu.VMEM((C, 128), F32),
        pltpu.VMEM((9 * NG + 1 + NT, 8, 128), F32),
    )


@jax.jit
def pallas_standalone__modern_conv_block_convnext_v2__vision_kernel(
    x: jax.Array,
    dw: jax.Array,
    w1: jax.Array,
    w2: jax.Array,
    grn_gamma: jax.Array,
    grn_beta: jax.Array,
):
    B, H, W, C = x.shape
    E = w1.shape[1]
    assert (B, W, C, E) == (1, 512, 96, 384) and dw.shape == (3, 3, C) and H % (2 * U1 * RB) == 0
    hbm = pl.BlockSpec(memory_space=pl.ANY)
    out = pl.pallas_call(
        _kernel,
        out_shape=jax.ShapeDtypeStruct((H, C, W), x.dtype),
        in_specs=[hbm] * 6,
        out_specs=hbm,
        scratch_shapes=[
            pltpu.VMEM((NX * RB, C, W), BF16),
            pltpu.VMEM((H // RB * (RB - NREC), W // 128, E, 128), BF16),
            pltpu.VMEM((E, 128), BF16),
            pltpu.VMEM((C, E), BF16),
            pltpu.VMEM((2, 1, E), F32),
            pltpu.VMEM(dw.shape, BF16),
            pltpu.VMEM((E,), BF16),
            pltpu.VMEM((E,), BF16),
            pltpu.SemaphoreType.DMA((NX,)),
            pltpu.SemaphoreType.DMA((NO,)),
            pltpu.SemaphoreType.DMA((3,)),
        ],
        compiler_params=pltpu.CompilerParams(vmem_limit_bytes=128 * 1024 * 1024, disable_bounds_checks=True),
        name="convnext_v2_block",
    )(jnp.transpose(x, (0, 1, 3, 2)).reshape(H, C, W), dw, w1, w2.T, grn_gamma, grn_beta)
    return jnp.transpose(out.reshape(B, H, C, W), (0, 1, 3, 2))
```

```python
import math

import jax
import jax.numpy as jnp
import jax.experimental.pallas as pl
import jax.experimental.pallas.tpu as pltpu

F32 = jnp.float32
BF16 = jnp.bfloat16
I32 = jnp.int32

RB = 8
NREC = 3
U1 = 4
NX = 5
NO = 2
RS = 9

LAG1 = 4
STATS_AT = 3
PIVOT_EVERY = 5
SEQ = "us" + "usd" * 11 + "ssd" + "s" * 6
LAG2 = 5
SIDE_FROM, SIDE_TO = 1, 29
CENTRE_AT = (2, 4, 6, 8)
FETCH_AT = 14

_C0 = math.sqrt(2.0 / math.pi)
_K = (_C0 * 0.044715) ** (1.0 / 3.0)
_B = _C0 / _K


def _gelu(z):
    return z * (jnp.tanh(z * (z * z + _B)) + 1.0)


def _ln_scale(var):
    return jax.lax.rsqrt(var + 1e-5) * _K


def _dot(lhs, rhs):
    return jnp.dot(lhs, rhs, preferred_element_type=F32)


def _pad_rows(v):
    return jnp.concatenate([v, jnp.zeros((128 - v.shape[0], v.shape[1]), v.dtype)], axis=0)


def _walsh(a, c):
    p = a & c & 7
    return (1 - 2 * ((p ^ (p >> 1) ^ (p >> 2)) & 1)).astype(F32)


def _tree_sum(parts):
    while len(parts) > 1:
        parts = [parts[i] + parts[i + 1] if i + 1 < len(parts) else parts[i] for i in range(0, len(parts), 2)]
    return parts[0]


def _tiles(v):
    return [v[:, c:c + 128] for c in range(0, v.shape[1], 128)]


def _neighbours(left, right):
    lane = jax.lax.broadcasted_iota(I32, (8, 128), 1)
    zero = jnp.zeros((8, 128), left[0].dtype)
    le = [zero] + [pltpu.roll(v, 1, 1) for v in left]
    ri = [pltpu.roll(v, 127, 1) for v in right] + [zero]
    return ([jnp.where(lane == 0, le[c], le[c + 1]) for c in range(len(left))],
            [jnp.where(lane == 127, ri[c + 1], ri[c]) for c in range(len(right))])


def _kernel(x_hbm, dw_hbm, w1_hbm, w2t_hbm, gamma_hbm, beta_hbm, o_hbm,
            xbuf, hbuf, w1t, wbuf, total, dw_ref, gamma_ref, beta_ref, isem, osem, wsem):
    H, C, W = x_hbm.shape
    E = w1_hbm.shape[1]
    NB = H // RB
    NG = C // 8
    NT = W // 128
    NST = RB - NREC
    rec_rows = list(range(1, 1 + NREC))
    st_rows = [r for r in range(RB) if r not in rec_rows]

    def next_slot(slot, n=1):
        return jnp.where(slot + n >= NX, slot + n - NX, slot + n)

    def x_copy(item, slot):
        row = jnp.where(item <= NB, jnp.minimum(item * RB - 1, H - RB), (item - NB - 1) * RB)
        return pltpu.make_async_copy(x_hbm.at[pl.ds(row, RB)], xbuf.at[pl.ds(slot * RB, RB)], isem.at[slot])

    def tap_columns():
        eye = jax.lax.broadcasted_iota(I32, (C, C), 0) == jax.lax.broadcasted_iota(I32, (C, C), 1)
        rows = [dw_ref[i].astype(F32) for i in range(3)]
        return [jnp.sum(jnp.where(eye, rows[i][j:j + 1, :], 0.0), axis=1, keepdims=True)
                for i in range(3) for j in range(3)]

    def pass1(sbuf, rbuf, scale, hnbuf, ssq, w1h, *cbufs):
        TAPS = 4 * NT
        hw = hnbuf.bitcast(I32)
        pace = []

        dw_copy = pltpu.make_async_copy(dw_hbm, dw_ref, wsem.at[0])
        w1_copy = pltpu.make_async_copy(w1_hbm, wbuf, wsem.at[1])
        head_copy = pltpu.make_async_copy(x_hbm.at[pl.ds(0, RB - 1)], xbuf.at[pl.ds(1, RB - 1)], isem.at[0])
        late_copies = [pltpu.make_async_copy(w2t_hbm, wbuf, wsem.at[0]),
                       pltpu.make_async_copy(gamma_hbm, gamma_ref, wsem.at[1]),
                       pltpu.make_async_copy(beta_hbm, beta_ref, wsem.at[2])]
        for cp in (dw_copy, w1_copy, head_copy, x_copy(1, 1)):
            cp.start()

        dw_copy.wait()
        taps = tap_columns()
        ro = jax.lax.broadcasted_iota(I32, (8, 128), 0)
        co = jax.lax.broadcasted_iota(I32, (8, 128), 1)
        for g in range(NG):
            halves = []
            for o in range(2):
                m = jnp.zeros((8, 128), F32)
                for i in range(3):
                    for j in range(3):
                        m = jnp.where(co == ro + (j * 32 + (i + o) * 8), taps[i * 3 + j][g * 8:(g + 1) * 8], m)
                halves.append(jnp.sum(m, axis=0, keepdims=True) * _walsh(ro, co))
            hnbuf[TAPS + g // 6, 16 * (g % 6):16 * (g % 6) + 16, :] = jnp.concatenate(halves, axis=0).astype(BF16)
        ssq[...] = jnp.zeros_like(ssq)
        xbuf[0] = jnp.zeros((C, W), BF16)

        head_copy.wait()
        w1_copy.wait()
        w1 = wbuf[...]
        w1t[...] = _pad_rows(w1.astype(F32)).T.astype(BF16)
        ra = jax.lax.broadcasted_iota(I32, (128, C), 0)
        ca = jax.lax.broadcasted_iota(I32, (128, C), 1)
        unmix = jnp.where((ra >> 3) == (ca >> 3), _walsh(ra, ca) * 0.125, 0.0).astype(BF16)
        row = jax.lax.broadcasted_iota(I32, (128, E), 0)
        mu = jnp.sum(w1.astype(F32), axis=0, keepdims=True) * (1.0 / C)
        mixed = _dot(unmix, w1) - jnp.where(((row & 7) == 0) & (row < C), mu, 0.0)
        w1h[...] = jnp.where(row == 0, 0.0, mixed).T.astype(BF16)
        for cp in late_copies:
            cp.start()

        def s_at(p, g, j, c):
            return ((p % 2) * NG + g) * 2 + c // 2, pl.ds(8 * (3 * (c % 2) + j), 8)

        def shift(slot, k, g):
            two_rows = xbuf[pl.ds(slot * RB + 2 * k, 2), 8 * g:8 * g + 8, :].reshape(16, W)
            mid = _tiles(pltpu.bitcast(two_rows, I32))
            left, right = _neighbours(mid, mid)
            for j, vs in enumerate((left, mid, right)):
                for c in range(NT):
                    sbuf[s_at(k, g, j, c)] = vs[c]

        def conv(q, g, acc, zero=0):
            rhs = jnp.concatenate([jnp.concatenate([sbuf[s_at(p, g, j, c)] for c in range(NT)], axis=1)
                                   for j in range(3) for p in (q, q + 1)], axis=0)
            lhs = pltpu.bitcast(hw[TAPS + g // 6 + zero, 8 * (g % 6):8 * (g % 6) + 8, :], BF16)
            y = _dot(lhs, _pad_rows(pltpu.bitcast(rhs, BF16)))
            for i, v in enumerate(_tiles(y[0:8]) + _tiles(y[8:16])):
                cbufs[q % 2][g, RS * i:RS * i + 8, :] = v
            pace.append(y[0:8, 0:128])
            if g == 0:
                return [y * y]
            acc = [acc[0] + y * y] + acc[1:]
            todo = [(h, zero) for h in range(max(g - PIVOT_EVERY, 1), g)] if g % PIVOT_EVERY == 0 else []
            if g == NG - 1:
                todo += [(h, 0) for h in range(g - g % PIVOT_EVERY, NG)]
            first = pl.ds(0, 8, stride=RS)
            es = [cbufs[q % 2][h + z, first, :] - cbufs[q % 2][0, first, :] for h, z in todo]
            for (h, _), e in zip(todo, es):
                cbufs[q % 2][h, first, :] = e
                acc = [acc[0], e, e * e] if h == 1 else [acc[0], acc[1] + e, acc[2] + e * e]
            if g == NG - 1:
                for i, v in enumerate(_tiles(acc[0][0:8]) + _tiles(acc[0][8:16])):
                    rbuf[RS * i:RS * i + 8, :] = v
                rbuf[RS * 8:RS * 8 + 8, :] = acc[2] - acc[1] * acc[1] * (1.0 / NG)
            return acc

        def ln_stats(q):
            squares = [rbuf[RS * 8:RS * 8 + 8, :]] + [rbuf[pl.ds(k, 8, stride=RS), :] for k in range(1, 8)]
            scale[q % 2] = _ln_scale(_tree_sum(squares) * (0.125 / C))

        def ln_apply(q, i, zero=0):
            if len(pace) >= LAG1:
                scale[2] = pace[-LAG1]
            d = cbufs[q % 2][:, RS * i:RS * i + 8, :] * scale[q % 2 + zero, i:i + 1, :]
            hnbuf[(q % 2) * 2 * NT + i] = d.reshape(C, 128).astype(BF16)

        def up(b0, j, q, g):
            o, e0 = g // (NG // 2), (g % (NG // 2)) * 64
            lhs = pltpu.bitcast(w1h.bitcast(I32)[e0 // 2:e0 // 2 + 32, :], BF16)
            hn = jnp.concatenate([hw[((q % 2) * 2 + o) * NT + c] for c in range(NT)], axis=1)
            a = _gelu(_dot(lhs, _pad_rows(pltpu.bitcast(hn, BF16))))
            ssq[e0:e0 + 64, :] += _tree_sum(_tiles(a * a))
            r = 2 * q + o
            if r in st_rows:
                for c, v in enumerate(_tiles(a)):
                    hbuf[(b0 + j) * NST + st_rows.index(r), c, e0:e0 + 64, :] = v.astype(BF16)

        for k in range(2):
            for g in range(NG):
                shift(0, k, g)
        for q in range(2):
            acc = None
            for g in range(NG):
                acc = conv(q, g, acc)
                shift(0, q + 2, g)
            if q == 0:
                ln_stats(0)
                for i in range(2 * NT):
                    ln_apply(0, i)

        def blocks(n, first):
            def body(t, slot):
                b0 = first + t * n
                slots = [next_slot(slot, j) for j in range(n + 1)]
                for j in range(1, n + 1):
                    x_copy(b0 + j, slots[j]).wait()
                if first > 0:
                    @pl.when(b0 + n == NB)
                    def _():
                        xbuf[slots[n] * RB] = xbuf[slots[n] * RB + RB - 1]
                        xbuf[slots[n] * RB + 1] = jnp.zeros((C, W), BF16)

                zero = t >> 16
                pace.clear()
                for j in range(n):
                    for k in range(RB // 2):
                        acc = None
                        for g in range(NG):
                            acc = conv(k + 2, g, acc, zero)
                            if g == STATS_AT:
                                ln_stats(k + 1)
                            if g > STATS_AT:
                                ln_apply(k + 1, g - STATS_AT - 1, zero)
                            if (k, g) == (0, 0):
                                x_copy(b0 + j + NX, slots[j]).start()
                            shift(slots[j + 1], k, g)
                            up(b0, j, k, g)
                return slots[n]
            return body

        for i in range(2, NX):
            x_copy(i, i).start()
        jax.lax.fori_loop(0, U1, blocks(1, 0), 0)
        jax.lax.fori_loop(0, NB // U1 - 1, blocks(U1, U1), U1 % NX)
        for cp in late_copies + [x_copy(NB + 1, (NB + 1) % NX)]:
            cp.wait()
        total[0] = jnp.sum(ssq[...].T, axis=0, keepdims=True)

    def pass2(obuf, cbuf, scale, bias, dwb):
        W2 = NREC * C
        ACC = W2 + C // 2
        MEAN = 9 * NG + 1

        def out_copy(b):
            return pltpu.make_async_copy(obuf.at[b % NO], o_hbm.at[pl.ds(b * RB, RB)], osem.at[b % NO])

        inv = 1.0 / (2.0 * _K)
        gx = jnp.sqrt(total[0] * (inv * inv) + 1e-6)
        nx = gx / (jnp.sum(gx, axis=1, keepdims=True) * (1.0 / E) + 1e-6)
        grn = (gamma_ref[...].astype(F32).reshape(1, E) * nx + 1.0) * inv
        for k, col in enumerate(tap_columns()):
            dwb[k * NG:(k + 1) * NG] = jnp.broadcast_to(col, (C, 128)).reshape(NG, 8, 128)
        w2t = wbuf[...].astype(F32)
        cbuf[W2:ACC, 0:E] = pltpu.bitcast((w2t * grn).astype(BF16), I32)
        beta = beta_ref[...].astype(F32).reshape(1, E)
        bias[...] = jnp.broadcast_to(jnp.sum(w2t * beta, axis=1, keepdims=True), (C, 128))

        def conv(slot, n, g, zero=0):
            xs = [xbuf[slot * RB + n + i, 8 * g:8 * g + 8, :].astype(F32) for i in range(3)]
            wt = [jnp.tile(dwb[k * NG + g + (zero if k < 3 else 0)], (1, NT)) for k in range(9)]
            p = [_tiles(xs[0] * wt[j] + xs[1] * wt[3 + j] + xs[2] * wt[6 + j]) for j in range(3)]
            left, right = _neighbours(p[0], p[2])
            y = jnp.concatenate([left[c] + p[1][c] + right[c] for c in range(NT)], axis=1)
            cbuf[n * C + 8 * g:n * C + 8 * g + 8, :] = pltpu.bitcast(y, I32)
            if g > 0:
                y = pltpu.bitcast(cbuf[ACC:ACC + 8, :], F32) + y
            if g < NG - 1:
                cbuf[ACC:ACC + 8, :] = pltpu.bitcast(y, I32)
            else:
                for c, v in enumerate(_tiles(jnp.sum(y, axis=0, keepdims=True) / C)):
                    dwb[MEAN + c] = jnp.broadcast_to(v, (8, 128))

        def centre(n, c, zero=0):
            rows, cols = slice(n * C, (n + 1) * C), slice(128 * c, 128 * c + 128)
            d = pltpu.bitcast(cbuf[rows, cols], F32) - jnp.tile(dwb[MEAN + c + zero], (NG, 1))
            cbuf[rows, cols] = pltpu.bitcast(d, I32)
            scale[n, :, cols] = _ln_scale(jnp.sum(d * d, axis=0, keepdims=True) * (1.0 / C))

        side = []
        for i in range(NREC):
            for g in range(NG):
                side.append(("conv", (i + NREC - 1) % NREC, g))
                if g in CENTRE_AT:
                    side.append(("centre", (i + NREC - 2) % NREC, CENTRE_AT.index(g)))
        cost = [0]
        for kind, _, _ in side:
            cost.append(cost[-1] + (3 if kind == "conv" else 1))
        side_at = [SIDE_FROM + v * (SIDE_TO - SIDE_FROM) // cost[-2] for v in cost[:-1]]
        for n in range(NREC - 1):
            for g in range(NG):
                conv((NB + 1) % NX, n, g)
            if n < NREC - 2:
                for c in range(NT):
                    centre(n, c)

        def body(b, slot):
            slot1, zero = next_slot(slot), b >> 16
            pl.when(b + 1 < NB)(lambda: x_copy(NB + 2 + b, slot1).wait())
            pl.when(b >= NO)(lambda: out_copy(b - NO).wait())
            acts, ys, pace = {}, {}, []

            def up(n, c):
                y = pltpu.bitcast(cbuf[n * C:(n + 1) * C, 128 * c:128 * c + 128], F32)
                hn = (y * scale[n, :, 128 * c:128 * c + 128]).astype(BF16)
                parts = []
                for k in range(E // C):
                    w = pltpu.bitcast(w1t.bitcast(I32)[C // 2 * k:C // 2 * (k + 1), :], BF16)[:, :C]
                    parts.append(_gelu(_dot(w, hn)))
                acts[n, c] = jnp.concatenate(parts, axis=0).astype(BF16)

            def down(r, c, a):
                i = len(pace)
                if i >= LAG2 and i in side_at:
                    dwb[9 * NG] = pace[-LAG2]
                for at, (kind, n, g) in zip(side_at, side):
                    if at == i and kind == "conv":
                        assert ((n, 0) not in acts) if n == NREC - 1 else ((n, NT - 1) in acts)
                        conv(slot if n == NREC - 1 else slot1, n, g, zero)
                    elif at == i:
                        assert ((n, g) not in acts) if n >= NREC - 2 else ((n, NT - 1) in acts)
                        centre(n, g, zero)
                if i == FETCH_AT:
                    pl.when(b + NX - 1 < NB)(lambda: x_copy(NB + b + NX, next_slot(slot, NX - 1)).start())
                w = jnp.concatenate([cbuf[pl.ds(pl.multiple_of(W2 + zero * 8, 8), 8), 0:E],
                                     cbuf[W2 + 8:ACC, 0:E]], axis=0)
                ys[r, c] = _dot(pltpu.bitcast(w, BF16), a)
                pace.append(ys[r, c][0:8])
                if c % 2 == 1:
                    cols = slice(128 * c - 128, 128 * c + 128)
                    res = jnp.tile(bias[...], (1, 2)) + xbuf[slot * RB + r, :, cols].astype(F32)
                    y = jnp.concatenate([ys[r, c - 1], ys[r, c]], axis=1)
                    obuf[b % NO, r, :, cols] = (y + res).astype(BF16)

            done = {"u": 0, "d": 0, "s": 0}
            for op in SEQ:
                n, c = divmod(done[op], NT)
                done[op] += 1
                if op == "u":
                    up(n, c)
                elif op == "d":
                    down(rec_rows[n], c, acts[n, c])
                else:
                    down(st_rows[n], c, pltpu.bitcast(hbuf.bitcast(I32)[b * NST + n, c], BF16))
            assert done == {"u": NT * NREC, "d": NT * NREC, "s": NT * NST}
            out_copy(b).start()
            return slot1

        jax.lax.fori_loop(0, NB, body, (NB + 1) % NX)
        for b in range(NB - NO, NB):
            out_copy(b).wait()

    pl.run_scoped(
        pass1,
        pltpu.VMEM((4 * NG, 48, 128), I32),
        pltpu.VMEM((8 * RS + 8, 128), F32),
        pltpu.VMEM((3, 8, 128), F32),
        pltpu.VMEM((4 * NT + 2, C, 128), BF16),
        pltpu.VMEM((E, 128), F32),
        pltpu.VMEM((E, 128), BF16),
        *[pltpu.VMEM((NG, 8 * RS, 128), F32)] * 2,
    )
    pl.run_scoped(
        pass2,
        pltpu.VMEM((NO, RB, C, W), BF16),
        pltpu.VMEM((NREC * C + C // 2 + 8, W), I32),
        pltpu.VMEM((NREC + 1, 1, W), F32),
        pltpu.VMEM((C, 128), F32),
        pltpu.VMEM((9 * NG + 1 + NT, 8, 128), F32),
    )


@jax.jit
def pallas_standalone__modern_conv_block_convnext_v2__vision_kernel(
    x: jax.Array,
    dw: jax.Array,
    w1: jax.Array,
    w2: jax.Array,
    grn_gamma: jax.Array,
    grn_beta: jax.Array,
):
    B, H, W, C = x.shape
    E = w1.shape[1]
    assert (B, W, C, E) == (1, 512, 96, 384) and dw.shape == (3, 3, C) and H % (U1 * RB) == 0 and H > NX * RB
    hbm = pl.BlockSpec(memory_space=pl.ANY)
    out = pl.pallas_call(
        _kernel,
        out_shape=jax.ShapeDtypeStruct((H, C, W), x.dtype),
        in_specs=[hbm] * 6,
        out_specs=hbm,
        scratch_shapes=[
            pltpu.VMEM((NX * RB, C, W), BF16),
            pltpu.VMEM((H // RB * (RB - NREC), W // 128, E, 128), BF16),
            pltpu.VMEM((E, 128), BF16),
            pltpu.VMEM((C, E), BF16),
            pltpu.VMEM((2, 1, E), F32),
            pltpu.VMEM(dw.shape, BF16),
            pltpu.VMEM((E,), BF16),
            pltpu.VMEM((E,), BF16),
            pltpu.SemaphoreType.DMA((NX,)),
            pltpu.SemaphoreType.DMA((NO,)),
            pltpu.SemaphoreType.DMA((3,)),
        ],
        compiler_params=pltpu.CompilerParams(vmem_limit_bytes=128 * 1024 * 1024, disable_bounds_checks=True),
        name="convnext_v2_block",
    )(jnp.transpose(x, (0, 1, 3, 2)).reshape(H, C, W), dw, w1, w2.T, grn_gamma, grn_beta)
    return jnp.transpose(out.reshape(B, H, C, W), (0, 1, 3, 2))
```
